```python
import os as _os
_os.environ.setdefault("JAX_PLATFORMS", "cpu")
import jax
import jax.numpy as jnp

def _softmax(x, axis=-1):
    return jax.nn.softmax(x, axis=axis)
def _gelu(x):
    return jax.nn.gelu(x, approximate=True)
def _silu(x):
    return jax.nn.silu(x)
def _sigmoid(x):
    return jax.nn.sigmoid(x)
def _layernorm(x, axis=-1, eps=1e-5):
    m = jnp.mean(x, axis=axis, keepdims=True)
    v = jnp.var(x, axis=axis, keepdims=True)
    return (x - m) / jnp.sqrt(v + eps)
def _scatter_add(tgt, idx, src, axis=0):
    return tgt.at[idx].add(src)
def _segment_sum(src, seg, n):
    return jax.ops.segment_sum(src, seg, n)
class _Rng:
    def __init__(self, key):
        self._k = key
    def _next(self):
        self._k, sub = jax.random.split(self._k)
        return sub
    def normal(self, shape):
        return jax.random.normal(self._next(), shape, dtype=jnp.bfloat16)
    def randint(self, lo, hi, shape):
        return jax.random.randint(self._next(), shape, lo, hi, dtype=jnp.int32)
    def uniform(self, shape, lo=0.0, hi=1.0):
        return jax.random.uniform(self._next(), shape, jnp.bfloat16, lo, hi)
    def permutation(self, n):
        return jax.random.permutation(self._next(), n)


kernel_name = 'parallel_sum__grouped_kv_mqa__dense_activation_silu__prompt'

def setup_inputs():
    _rng = _Rng(jax.random.key(int.from_bytes(__import__("os").urandom(4), "little")))
    _w = (lambda a: (lambda t: t.astype(jnp.bfloat16) if jnp.issubdtype(t.dtype, jnp.floating) else t)(jnp.asarray(a)))
    def _A_setup():
        B, S, D, H = 1, 2048, 512, 32
        Dh = D // H
        return {
            "x": _w((lambda *s: _rng.normal(s) * 0.05)(B, S, D)),
            "wq": _w((lambda *s: _rng.normal(s) * 0.05)(D, H * Dh)),
            "wk": _w((lambda *s: _rng.normal(s) * 0.05)(D, Dh)),
            "wv": _w((lambda *s: _rng.normal(s) * 0.05)(D, Dh)),
            "wo": _w((lambda *s: _rng.normal(s) * 0.05)(H * Dh, D)),
        }
    _A_in = _A_setup()

    def _B_setup():
        B, S, D, F = 1, 2048, 512, 1376
        return {
            "x": _w((lambda *s: _rng.normal(s) * 0.05)(B, S, D)),
            "w1": _w((lambda *s: _rng.normal(s) * 0.05)(D, F) * (D ** -0.5)),
            "w2": _w((lambda *s: _rng.normal(s) * 0.05)(F, D) * (F ** -0.5)),
        }
    _B_in = _B_setup()

    return {
        "A_x": _A_in["x"],
        "A_wq": _A_in["wq"],
        "A_wk": _A_in["wk"],
        "A_wv": _A_in["wv"],
        "A_wo": _A_in["wo"],
        "B_x": _B_in["x"],
        "B_w1": _B_in["w1"],
        "B_w2": _B_in["w2"],
    }

def reference(A_x, A_wq, A_wk, A_wv, A_wo, B_x, B_w1, B_w2):
    def _A_ref(x, wq, wk, wv, wo):
        B, S, D = x.shape
        H = 32
        Dh = D // H
        q = (lambda x, *d: x.transpose(*d))((x @ wq).reshape(B, S, H, Dh), 0, 2, 1, 3)
        k = x @ wk
        v = x @ wv
        scores = jnp.einsum("bhqd,bkd->bhqk", q, k) * (Dh ** -0.5)
        p = _softmax(scores, axis=-1)
        o = jnp.einsum("bhqk,bkd->bhqd", p, v)
        return (lambda x, *d: x.transpose(*d))(o, 0, 2, 1, 3).reshape(B, S, H * Dh) @ wo

    def _B_ref(x, w1, w2):
        h = jnp.einsum("bsd,df->bsf", x, w1)
        h = _silu(h)
        out = jnp.einsum("bsf,fd->bsd", h, w2)
        return out

    x = A_x
    xn = _layernorm(x, axis=-1)
    return x + _A_ref(xn, A_wq, A_wk, A_wv, A_wo) + _B_ref(xn, B_w1, B_w2)
```

```python
import math

import jax
import jax.numpy as jnp
import numpy as np
from jax import lax
import jax.experimental.pallas as pl
import jax.experimental.pallas.tpu as pltpu

S, D, H, DH, F = 2048, 512, 32, 16, 1376
TQ = 512
NT = S // TQ
NU = NT * H
KC = 128
NK = S // KC
NC = TQ // 128
DE = 32
QSCALE = (DH ** -0.5) * math.log2(math.e)
UP = 1.0 + 2.0 ** -6
L_MIN = 2.0 ** -60
EPS = 1e-5
f32, bf16, u32 = jnp.float32, jnp.bfloat16, jnp.uint32
NT_DIMS = (((1,), (1,)), ((), ()))
TN_DIMS = (((0,), (0,)), ((), ()))

G = 4
NVL = [16] * 14 + [0] * 2
LEAD = 8
ROT = 8
S0, S1 = 0.0, 8.0

GOFF = [int(v) for v in np.concatenate([[0], np.cumsum(NVL)]) // 8]
NV = int(sum(NVL))
NBL = [(KC - v) // 16 for v in NVL]
BOFF = [int(v) for v in np.concatenate([[0], np.cumsum(NBL)])]
NB = BOFF[-1]
NG = NV // 8
TILE_OF_GROUP = [j for j in range(NK) for _ in range(NVL[j] // 8)]
ALLP = [(g, r, c) for g in range(G) for r in range(NG) for c in range(NC)]
_LO, _HI = int((ROT + S0) * 8), int((G * NB + ROT - S1) * 8)
PTS = [min(_HI - 1, int(_LO + n * (_HI - _LO) / len(ALLP))) for n in range(len(ALLP))]
NI = NU // G


def _kernel(x_hbm, wq_hbm, wkt_hbm, wvt_hbm, wo_hbm, w1t_hbm, w2_hbm, o_hbm,
            x_ref, wq_ref, wt_ref, wo_ref, w1t_ref, w2_ref, o_ref,
            xn_ref, qt_ref, qf_ref, nrm_ref, bias_ref, kx_ref, kn_ref, kv_ref, kb_ref,
            vt_ref, ot_ref, pvs_ref, pre_ref, zf_ref, z_ref,
            sem_x, sem_w, sem_o):
    x_cp = [pltpu.make_async_copy(x_hbm.at[pl.ds(t * TQ, TQ)], x_ref.at[pl.ds(t * TQ, TQ)], sem_x.at[t])
            for t in range(NT)]
    w_cp = [pltpu.make_async_copy(a, b, sem_w.at[i]) for i, (a, b) in enumerate(
        [(wq_hbm, wq_ref), (wkt_hbm, wt_ref.at[pl.ds(D, DH)]), (wvt_hbm, wt_ref.at[pl.ds(D + DH, DH)]),
         (w1t_hbm, w1t_ref), (w2_hbm, w2_ref), (wo_hbm, wo_ref)])]
    for c in w_cp[:3]:
        c.start()
    x_cp[0].start()
    x_cp[1].start()
    zf_ref[...] = jnp.zeros(zf_ref.shape, f32)
    z_ref[...] = jnp.zeros(z_ref.shape, u32)

    row16 = lax.broadcasted_iota(jnp.int32, (DH, TQ), 0)
    row8 = lax.broadcasted_iota(jnp.int32, (8, TQ), 0)

    def layernorm(t):
        x = x_ref[t * TQ:(t + 1) * TQ, :].astype(f32)
        mu = jnp.mean(x, axis=-1, keepdims=True)
        xc = x - mu
        var = jnp.mean(xc * xc, axis=-1, keepdims=True)
        xn_ref[t * TQ:(t + 1) * TQ, :] = (xc * lax.rsqrt(var + EPS)).astype(bf16)

    def proj_kv(t):
        xn = xn_ref[t * TQ:(t + 1) * TQ, :]
        r = lax.dot_general(wt_ref[D:D + 2 * DH, :], xn, NT_DIMS, preferred_element_type=f32)
        kt = r[0:DH].astype(bf16).astype(f32)
        vt_ref[:, t * TQ:(t + 1) * TQ] = r[DH:].astype(bf16)
        k2 = jnp.sum(kt * kt, axis=0, keepdims=True)
        ones_row = jnp.where(row16 == 0, 1.0, 0.0).astype(f32)
        ke = jnp.concatenate([kt, ones_row], axis=0).T
        kn_ref[t * TQ:(t + 1) * TQ, :] = ke.astype(bf16)
        for jj in range(TQ // KC):
            j = t * (TQ // KC) + jj
            for b in range(NBL[j]):
                src = jj * KC + NVL[j] + 16 * (NBL[j] - 1 - b)
                kx_ref[8 * (BOFF[j] + b): 8 * (BOFF[j] + b) + 8, :] = pltpu.bitcast(
                    ke[src:src + 16, :].astype(bf16), u32)
            if NVL[j]:
                kv_ref[GOFF[j] * 8: GOFF[j] * 8 + NVL[j], :] = ke[jj * KC: jj * KC + NVL[j], :].astype(bf16)
            for r0 in range(0, NVL[j], 8):
                kv = ke[jj * KC + r0: jj * KC + r0 + 8, :]
                for d in range(DH):
                    kb_ref[d, GOFF[j] * 8 + r0: GOFF[j] * 8 + r0 + 8, :] = jnp.broadcast_to(
                        kv[:, d:d + 1], (8, 128))
        return k2

    def proj_q(t):
        xn = xn_ref[t * TQ:(t + 1) * TQ, :]
        r = lax.dot_general(wt_ref[0:D, :], xn, NT_DIMS, preferred_element_type=f32)
        qb = (r * QSCALE).astype(bf16)
        qf = qb.astype(f32).reshape(H, DH, TQ)
        qt_ref[t * H:(t + 1) * H] = qb.reshape(H, DH, TQ)
        qf_ref[t * H:(t + 1) * H] = qf
        nrm_ref[t * H:(t + 1) * H, :] = jnp.sum(qf * qf, axis=1)

    def put_bias(t, kmax2):
        bias = (jnp.sqrt(nrm_ref[t * H:(t + 1) * H, :] * kmax2) * (-UP)).astype(bf16).astype(f32)
        for k in range(H // G):
            bias_ref[t * (H // G) + k, 0:G, :] = bias[k * G:(k + 1) * G]

    def q_ext(it, g):
        brow = jnp.broadcast_to(bias_ref[it, g:g + 1, :], (8, TQ))
        blk = jnp.concatenate([jnp.where(row8 == 0, brow, 0.0), jnp.zeros((8, TQ), f32)], axis=0)
        return jnp.concatenate([qt_ref[G * it + g], blk.astype(bf16)], axis=0)

    for c in w_cp[:3]:
        c.wait()
    wt_ref[0:D, :] = wq_ref[...].T
    x_cp[0].wait()
    x_cp[2].start()
    x_cp[3].start()
    layernorm(0)
    x_cp[1].wait()
    layernorm(1)
    k2 = proj_kv(0)
    proj_q(0)
    x_cp[2].wait()
    x_cp[3].wait()
    for c in w_cp[3:]:
        c.start()
    k2 = jnp.maximum(k2, proj_kv(1))
    layernorm(2)
    proj_q(1)
    k2 = jnp.maximum(k2, proj_kv(2))
    layernorm(3)
    k2 = jnp.maximum(k2, proj_kv(3))
    kmax2 = jnp.max(k2, axis=1, keepdims=True)
    put_bias(0, kmax2)
    put_bias(1, kmax2)
    proj_q(2)
    put_bias(2, kmax2)
    proj_q(3)
    put_bias(3, kmax2)

    def kblocks(b0, b1):
        return pltpu.bitcast(kx_ref[8 * b0:8 * b1, :], bf16)

    for g in range(G):
        pvs_ref[g] = jnp.exp2(jnp.dot(kv_ref[...], q_ext(0, g), preferred_element_type=f32))
    pre_ref[...] = jnp.exp2(jnp.dot(kblocks(0, ROT), q_ext(0, 0), preferred_element_type=f32))

    def stage(i, bad):
        L = [None] * G
        ACC = [None] * G
        Q = [None] * (G + 1)
        PM, SS = {}, {}
        done_v = set()
        st = dict(nextp=0, pos=ROT, bad=bad)
        never = z_ref[...] != 0
        inext = jnp.minimum(i + 1, NI - 1)

        def piece(g, r, c, lk):
            u = G * inext + g
            acc = jnp.broadcast_to(bias_ref[inext, g:g + 1, c * 128:(c + 1) * 128], (8, 128))
            acc = jnp.where(never, lk, acc)
            for d in range(DH):
                qb = jnp.broadcast_to(qf_ref[u, d:d + 1, c * 128:(c + 1) * 128], (8, 128))
                acc = acc + kb_ref[d, r * 8:r * 8 + 8, :] * qb
            pvs_ref[g, r * 8:r * 8 + 8, c * 128:(c + 1) * 128] = jnp.exp2(acc)

        def score(g, b0, b1):
            if Q[g] is None:
                Q[g] = q_ext(i, g) if g < G else q_ext(inext, 0)
            s = jnp.dot(kblocks(b0, b1), Q[g], preferred_element_type=f32)
            p = jnp.exp2(s)
            if g == G:
                pre_ref[16 * b0:16 * b1, :] = p
            for b in range(b0, b1):
                PM[(g, b)] = p[16 * (b - b0):16 * (b - b0) + 16]
                SS[g * NB + b] = s[16 * (b - b0):16 * (b - b0) + 16]

        def emit_pieces():
            while st["nextp"] < len(ALLP):
                g, r, c = ALLP[st["nextp"]]
                x = PTS[st["nextp"]]
                if (x // 8) not in SS or (g, TILE_OF_GROUP[r]) not in done_v:
                    break
                hf, cc = (x % 8) // 4, x % 4
                piece(g, r, c, SS[x // 8][8 * hf:8 * hf + 8, cc * 128:(cc + 1) * 128])
                st["nextp"] += 1

        def pv(g, j):
            blocks = [(pre_ref[16 * b:16 * b + 16, :] if (g == 0 and b < ROT) else PM.pop((g, b)))
                      for b in range(BOFF[j], BOFF[j + 1])]
            rows = [pvs_ref[g, r * 8:r * 8 + 8, :] for r in range(GOFF[j], GOFF[j + 1])]
            for x in blocks:
                for y in (x[0:8], x[8:16]):
                    L[g] = y if L[g] is None else L[g] + y
            for x in reversed(rows):
                L[g] = L[g] + x
            pb = jnp.concatenate(rows + blocks[::-1], axis=0).astype(bf16)
            o = jnp.dot(vt_ref[:, j * KC:(j + 1) * KC], pb, preferred_element_type=f32)
            if ACC[g] is None:
                ACC[g] = zf_ref[...]
            ACC[g] = ACC[g] + o
            if j == NK - 1:
                lsum = jnp.sum(L[g], axis=0, keepdims=True)
                ot_ref[G * i + g] = (ACC[g] / lsum).astype(bf16)
                st["bad"] = jnp.where(lsum >= L_MIN, st["bad"], 1.0)
            done_v.add((g, j))
            emit_pieces()

        def issue_to(p1):
            p1 = min(p1, G * NB + ROT)
            while st["pos"] < p1:
                g = st["pos"] // NB
                e = min(p1, (g + 1) * NB)
                score(g, st["pos"] - g * NB, e - g * NB)
                st["pos"] = e

        for g in range(G):
            for j in range(NK):
                issue_to(g * NB + BOFF[j + 1] + LEAD)
                pv(g, j)
        issue_to(G * NB + ROT)
        emit_pieces()
        assert st["nextp"] == len(ALLP)
        return st["bad"]

    bad = lax.fori_loop(0, NI, stage, jnp.zeros((1, TQ), f32))

    @pl.when(jnp.max(bad) > 0.0)
    def _():
        def unit(u, c):
            s = jnp.dot(kn_ref[:, 0:DH], qt_ref[u], preferred_element_type=f32)
            m = jnp.max(s, axis=0, keepdims=True)
            p = jnp.exp2(s - m)
            l = jnp.sum(p, axis=0, keepdims=True)
            o = jnp.dot(vt_ref[...], p.astype(bf16), preferred_element_type=f32)
            ot_ref[u] = (o / l).astype(bf16)
            return c
        lax.fori_loop(0, NU, unit, 0)

    for c in w_cp[3:]:
        c.wait()

    def o_cp(t):
        return pltpu.make_async_copy(o_ref.at[pl.ds(t * TQ, TQ)], o_hbm.at[pl.ds(t * TQ, TQ)], sem_o.at[t])

    def tile2(t, c):
        rows = pl.ds(pl.multiple_of(t * TQ, TQ), TQ)
        xn = xn_ref[rows, :]
        h = lax.dot_general(xn, w1t_ref[...], NT_DIMS, preferred_element_type=f32)
        h = (h * jax.nn.sigmoid(h)).astype(bf16)
        y = jnp.dot(h, w2_ref[...], preferred_element_type=f32)
        ot = ot_ref[pl.ds(t * H, H)].reshape(H * DH, TQ)
        y = y + lax.dot_general(ot, wo_ref[...], TN_DIMS, preferred_element_type=f32)
        o_ref[rows, :] = (x_ref[rows, :].astype(f32) + y).astype(bf16)
        o_cp(t).start()
        return c

    lax.fori_loop(0, NT, tile2, 0)
    for t in range(NT):
        o_cp(t).wait()


@jax.jit
def pallas_parallel_sum__grouped_kv_mqa__dense_activation_silu__prompt_kernel(
    A_x: jax.Array,
    A_wq: jax.Array,
    A_wk: jax.Array,
    A_wv: jax.Array,
    A_wo: jax.Array,
    B_x: jax.Array,
    B_w1: jax.Array,
    B_w2: jax.Array,
):
    del B_x
    anyspec = pl.BlockSpec(memory_space=pl.ANY)
    out = pl.pallas_call(
        _kernel,
        out_shape=jax.ShapeDtypeStruct((S, D), bf16),
        in_specs=[anyspec] * 7,
        out_specs=anyspec,
        scratch_shapes=[
            pltpu.VMEM((S, D), bf16),
            pltpu.VMEM((D, D), bf16),
            pltpu.VMEM((D + 2 * DH, D), bf16),
            pltpu.VMEM((D, D), bf16),
            pltpu.VMEM((F, D), bf16),
            pltpu.VMEM((F, D), bf16),
            pltpu.VMEM((S, D), bf16),
            pltpu.VMEM((S, D), bf16),
            pltpu.VMEM((NU, DH, TQ), bf16),
            pltpu.VMEM((NU, DH, TQ), f32),
            pltpu.VMEM((NU, TQ), f32),
            pltpu.VMEM((NI, 8, TQ), f32),
            pltpu.VMEM((NB * 8, DE), u32),
            pltpu.VMEM((S, DE), bf16),
            pltpu.VMEM((NV, DE), bf16),
            pltpu.VMEM((DH, NV, 128), f32),
            pltpu.VMEM((DH, S), bf16),
            pltpu.VMEM((NU, DH, TQ), bf16),
            pltpu.VMEM((G, NV, TQ), f32),
            pltpu.VMEM((ROT * 16, TQ), f32),
            pltpu.VMEM((DH, TQ), f32),
            pltpu.VMEM((8, 128), u32),
            pltpu.SemaphoreType.DMA((NT,)),
            pltpu.SemaphoreType.DMA((6,)),
            pltpu.SemaphoreType.DMA((NT,)),
        ],
        compiler_params=pltpu.CompilerParams(vmem_limit_bytes=100 * 1024 * 1024),
    )(A_x.reshape(S, D), A_wq, A_wk.T, A_wv.T, A_wo, B_w1.T, B_w2)
    return out.reshape(1, S, D)
```

```python
import math

import jax
import jax.numpy as jnp
import numpy as np
from jax import lax
import jax.experimental.pallas as pl
import jax.experimental.pallas.tpu as pltpu

S, D, H, DH, F = 2048, 512, 32, 16, 1376
TQ = 512
NT = S // TQ
NU = NT * H
KC = 128
NK = S // KC
NC = TQ // 128
DE = 32
QSCALE = (DH ** -0.5) * math.log2(math.e)
UP = 1.0 + 2.0 ** -6
L_MIN = 2.0 ** -60
EPS = 1e-5
f32, bf16, u32 = jnp.float32, jnp.bfloat16, jnp.uint32
NT_DIMS = (((1,), (1,)), ((), ()))
TN_DIMS = (((0,), (0,)), ((), ()))
FT = [(a, min(a + 128, F)) for a in range(0, F, 128)]

G = 8
NVL = [16] * 16
NXL = [16, 0, 0, 0, 0] * 3 + [0]
LEAD = 8
ROT = 8
S1 = 8
W1FRAC, F0, F1 = 0.55, 0.01, 0.03
LN_AHEAD = 3
OSPLIT = 4


def _offsets(counts, div):
    return [int(v) // div for v in np.concatenate([[0], np.cumsum(counts)])]


GOFF, XOFF = _offsets(NVL, 8), _offsets(NXL, 8)
NV, NX = int(sum(NVL)), int(sum(NXL))
NBL = [(KC - v - w) // 16 for v, w in zip(NVL, NXL)]
BOFF = _offsets(NBL, 1)
NB = BOFF[-1]
NG, NGX = NV // 8, NX // 8
TILE_OF_GROUP = [j for j in range(NK) for _ in range(NVL[j] // 8)]
ALLP = [(g, r0 + r, c) for g in range(G) for r0 in range(0, NG, 2) for c in range(NC) for r in range(2)]
_LO, _HI = ROT * 8, (G * NB + ROT - S1) * 8
PTS = [min(_HI - 1, int(_LO + n * (_HI - _LO) / len(ALLP))) for n in range(len(ALLP))]
NI = NU // G
XP = [(h, r0 + r, c) for h in range(H) for r0 in range(0, NGX, 2) for c in range(NC) for r in range(2)]
XN1 = int(len(XP) * W1FRAC)
XP1 = [int((F0 + (1 - F0) * n / XN1) * len(FT) * (TQ // 8)) for n in range(XN1)]
XP2 = [int((1 - F1) * n / (len(XP) - XN1) * len(FT) * (TQ // 8) * NC) for n in range(len(XP) - XN1)]
OSEG = ([(t * TQ, (t + 1) * TQ) for t in range(NT - 1)]
        + [((NT - 1) * TQ + k * (TQ // OSPLIT), (NT - 1) * TQ + (k + 1) * (TQ // OSPLIT)) for k in range(OSPLIT)])


def _kernel(x_hbm, wq_hbm, wkt_hbm, wvt_hbm, wo_hbm, w1t_hbm, w2_hbm, o_hbm,
            x_ref, wq_ref, wt_ref, wo_ref, w1t_ref, w2_ref, o_ref,
            xn_ref, qt_ref, qf_ref, nrm_ref, bias_ref, kx_ref, kn_ref, kv_ref, kb_ref,
            vt_ref, ot_ref, pvs_ref, pre_ref, px_ref, y_ref, ya_ref, h_ref, zf_ref, z_ref,
            sem_x, sem_w, sem_o):
    x_cp = [pltpu.make_async_copy(x_hbm.at[pl.ds(t * TQ, TQ)], x_ref.at[pl.ds(t * TQ, TQ)], sem_x.at[t])
            for t in range(NT)]
    w_cp = [pltpu.make_async_copy(a, b, sem_w.at[i]) for i, (a, b) in enumerate(
        [(wq_hbm, wq_ref), (wkt_hbm, wt_ref.at[pl.ds(D, DH)]), (wvt_hbm, wt_ref.at[pl.ds(D + DH, DH)]),
         (w1t_hbm, w1t_ref), (w2_hbm, w2_ref), (wo_hbm, wo_ref)])]
    for c in w_cp[:3]:
        c.start()
    x_cp[0].start()
    x_cp[1].start()
    zf_ref[...] = jnp.zeros(zf_ref.shape, f32)
    z_ref[...] = jnp.zeros(z_ref.shape, u32)

    row16 = lax.broadcasted_iota(jnp.int32, (DH, TQ), 0)
    row8 = lax.broadcasted_iota(jnp.int32, (8, TQ), 0)

    def layernorm(s, lk=None):
        x = x_ref[s * 128:(s + 1) * 128, :].astype(f32)
        if lk is not None:
            never = jnp.concatenate([z_ref[...] != 0] * 16, axis=0)
            x = jnp.concatenate([jnp.where(never, lk, x[:, 0:128]), x[:, 128:]], axis=1)
        mu = jnp.mean(x, axis=-1, keepdims=True)
        xc = x - mu
        var = jnp.mean(xc * xc, axis=-1, keepdims=True)
        xn_ref[s * 128:(s + 1) * 128, :] = (xc * lax.rsqrt(var + EPS)).astype(bf16)

    def proj_kv(t):
        xn = xn_ref[t * TQ:(t + 1) * TQ, :]
        r = lax.dot_general(wt_ref[D:D + 2 * DH, :], xn, NT_DIMS, preferred_element_type=f32)
        kt = r[0:DH].astype(bf16).astype(f32)
        vt_ref[:, t * TQ:(t + 1) * TQ] = r[DH:].astype(bf16).astype(f32)
        k2 = jnp.sum(kt * kt, axis=0, keepdims=True)
        ones_row = jnp.where(row16 == 0, 1.0, 0.0).astype(f32)
        ke = jnp.concatenate([kt, ones_row], axis=0).T
        kn_ref[t * TQ:(t + 1) * TQ, :] = ke.astype(bf16)
        for jj in range(TQ // KC):
            j = t * (TQ // KC) + jj
            for b in range(NBL[j]):
                src = jj * KC + NVL[j] + NXL[j] + 16 * (NBL[j] - 1 - b)
                kx_ref[8 * (BOFF[j] + b): 8 * (BOFF[j] + b) + 8, :] = pltpu.bitcast(
                    ke[src:src + 16, :].astype(bf16), u32)
            if NVL[j]:
                kv_ref[GOFF[j] * 8: GOFF[j] * 8 + NVL[j], :] = ke[jj * KC: jj * KC + NVL[j], :].astype(bf16)
            for r0 in range(0, NVL[j] + NXL[j], 8):
                kv = ke[jj * KC + r0: jj * KC + r0 + 8, :]
                dst = GOFF[j] * 8 + r0 if r0 < NVL[j] else NV + XOFF[j] * 8 + r0 - NVL[j]
                for d in range(DH):
                    kb_ref[d, dst:dst + 8, :] = jnp.broadcast_to(kv[:, d:d + 1], (8, 128))
        return k2

    def proj_q(s):
        t, a = s // NC, (s % NC) * 128
        xn = xn_ref[s * 128:(s + 1) * 128, :]
        r = lax.dot_general(wt_ref[0:D, :], xn, NT_DIMS, preferred_element_type=f32)
        qb = (r * QSCALE).astype(bf16)
        qf = qb.astype(f32).reshape(H, DH, 128)
        qt_ref[t * H:(t + 1) * H, :, a:a + 128] = qb.reshape(H, DH, 128)
        qf_ref[t * H:(t + 1) * H, :, a:a + 128] = qf
        nrm_ref[t * H:(t + 1) * H, a:a + 128] = jnp.sum(qf * qf, axis=1)
        return r

    def q_ext(it, g):
        brow = jnp.broadcast_to(bias_ref[it, g:g + 1, :], (8, TQ))
        blk = jnp.concatenate([jnp.where(row8 == 0, brow, 0.0), jnp.zeros((8, TQ), f32)], axis=0)
        return jnp.concatenate([qt_ref[G * it + g], blk.astype(bf16)], axis=0)

    for c in w_cp[:3]:
        c.wait()
    wt_ref[0:D, :] = wq_ref[...].T
    x_cp[0].wait()
    for c in x_cp[2:]:
        c.start()
    for s in range(NC):
        layernorm(s)
    for s in range(NC - 1):
        proj_q(s)
    for c in x_cp[1:]:
        c.wait()
    for c in w_cp[3:]:
        c.start()
    k2 = proj_kv(0)
    outs = {}
    nln = NC
    for s in range(NC - 1, NT * NC):
        while nln < NT * NC and nln - LN_AHEAD < s:
            lk = outs.get(nln - LN_AHEAD)
            if lk is not None:
                lk = jnp.concatenate([lk[32 * n:32 * n + 8] for n in range(16)], axis=0)
            layernorm(nln, lk)
            nln += 1
        if s % NC == NC - 1 and s >= NC:
            k2 = jnp.maximum(k2, proj_kv(s // NC))
        outs[s] = proj_q(s)
    kscale = jnp.sqrt(jnp.max(k2, axis=1, keepdims=True)) * (-UP)
    for t in range(NT):
        bias = (jnp.sqrt(nrm_ref[t * H:(t + 1) * H, :]) * kscale).astype(bf16).astype(f32)
        for k in range(H // G):
            bias_ref[t * (H // G) + k] = bias[k * G:(k + 1) * G]

    def vpu_probs(never, it, g, krow, c, lk):
        u = G * it + g
        acc = jnp.broadcast_to(bias_ref[it, g:g + 1, c * 128:(c + 1) * 128], (8, 128))
        acc = jnp.where(never, lk, acc)
        for d in range(DH):
            qb = jnp.broadcast_to(qf_ref[u, d:d + 1, c * 128:(c + 1) * 128], (8, 128))
            acc = acc + kb_ref[d, krow * 8:krow * 8 + 8, :] * qb
        return jnp.exp2(acc)

    def kblocks(b0, b1):
        return pltpu.bitcast(kx_ref[8 * b0:8 * b1, :], bf16)

    pvs_ref[0] = jnp.exp2(jnp.dot(kv_ref[...], q_ext(0, 0), preferred_element_type=f32))
    pre_ref[...] = jnp.exp2(jnp.dot(kblocks(0, ROT), q_ext(0, 0), preferred_element_type=f32))

    w_cp[3].wait()
    w_cp[4].wait()

    def ffn(t, carry):
        rows = pl.ds(pl.multiple_of(t * TQ, TQ), TQ)
        never = z_ref[...] != 0
        xn = xn_ref[rows, :]
        k = [0]

        def emit(lk):
            h, r, c = XP[k[0]]
            px_ref[t * H + h, r * 8:r * 8 + 8, c * 128:(c + 1) * 128] = vpu_probs(
                never, t * (H // G) + h // G, h % G, NG + r, c, lk)
            k[0] += 1

        for n, (a, b) in enumerate(FT):
            h = lax.dot_general(xn, w1t_ref[a:b, :], NT_DIMS, preferred_element_type=f32)
            hh = h * 0.5
            h_ref[:, a:b] = (hh + hh * jnp.tanh(hh)).astype(bf16)
            while k[0] < XN1 and XP1[k[0]] // (TQ // 8) == n:
                rg = XP1[k[0]] % (TQ // 8)
                hv = h[rg * 8:rg * 8 + 8, :]
                if b - a < 128:
                    hv = jnp.concatenate([hv, hv[:, 0:128 - (b - a)]], axis=1)
                emit(hv)
        for n, (a, b) in enumerate(FT):
            part = jnp.dot(h_ref[:, a:b], w2_ref[a:b, :], preferred_element_type=f32)
            if n == 0:
                ya_ref[...] = x_ref[rows, :].astype(f32) + part
            elif n == len(FT) - 1:
                y_ref[rows, :] = ya_ref[...] + part
            else:
                ya_ref[...] += part
            while k[0] < len(XP) and XP2[k[0] - XN1] // (TQ // 8 * NC) == n:
                v = XP2[k[0] - XN1] % (TQ // 8 * NC)
                rg, cc = v // NC, v % NC
                emit(part[rg * 8:rg * 8 + 8, cc * 128:(cc + 1) * 128])
        assert k[0] == len(XP)
        return carry

    lax.fori_loop(0, NT, ffn, 0)

    def stage(i, bad):
        L = [None] * G
        ACC = [None] * G
        Q = [None] * (G + 1)
        PM, SS = {}, {}
        done_v = set()
        st = dict(nextp=0, pos=ROT, bad=bad)
        never = z_ref[...] != 0
        inext = jnp.minimum(i + 1, NI - 1)

        def emit_pieces():
            while st["nextp"] < len(ALLP):
                g, r, c = ALLP[st["nextp"]]
                x = PTS[st["nextp"]]
                if (x // 8) not in SS or (g >= 1 and (g - 1, TILE_OF_GROUP[r]) not in done_v):
                    break
                hf, cc = (x % 8) // 4, x % 4
                it2, g2 = (i, g + 1) if g + 1 < G else (inext, 0)
                pvs_ref[g2 % 2, r * 8:r * 8 + 8, c * 128:(c + 1) * 128] = vpu_probs(
                    never, it2, g2, r, c, SS[x // 8][8 * hf:8 * hf + 8, cc * 128:(cc + 1) * 128])
                st["nextp"] += 1

        def score(g, b0, b1):
            if Q[g] is None:
                Q[g] = q_ext(i, g) if g < G else q_ext(inext, 0)
            s = jnp.dot(kblocks(b0, b1), Q[g], preferred_element_type=f32)
            p = jnp.exp2(s)
            if g == G:
                pre_ref[16 * b0:16 * b1, :] = p
            for b in range(b0, b1):
                PM[(g, b)] = p[16 * (b - b0):16 * (b - b0) + 16]
                SS[g * NB + b] = s[16 * (b - b0):16 * (b - b0) + 16]

        def pv(g, j):
            blocks = [(pre_ref[16 * b:16 * b + 16, :] if (g == 0 and b < ROT) else PM.pop((g, b)))
                      for b in range(BOFF[j], BOFF[j + 1])]
            if g >= 1:
                assert all((g - 1, r, c) in ALLP[:st["nextp"]]
                           for r in range(GOFF[j], GOFF[j + 1]) for c in range(NC))
            rows = [pvs_ref[g % 2, r * 8:r * 8 + 8, :] for r in range(GOFF[j], GOFF[j + 1])]
            rows += [px_ref[G * i + g, r * 8:r * 8 + 8, :] for r in range(XOFF[j], XOFF[j + 1])]
            for x in blocks:
                for y in (x[8:16], x[0:8]):
                    L[g] = y if L[g] is None else L[g] + y
            for x in reversed(rows):
                L[g] = L[g] + x
            pb = jnp.concatenate(rows + blocks[::-1], axis=0)
            o = jnp.dot(vt_ref[:, j * KC:(j + 1) * KC], pb, preferred_element_type=f32)
            if ACC[g] is None:
                ACC[g] = zf_ref[...]
            ACC[g] = ACC[g] + o
            if j == NK - 1:
                lsum = jnp.sum(L[g], axis=0, keepdims=True)
                ot_ref[G * i + g] = (ACC[g] / lsum).astype(bf16)
                st["bad"] = jnp.where(lsum >= L_MIN, st["bad"], 1.0)
            done_v.add((g, j))
            emit_pieces()

        def issue_to(p1):
            p1 = min(p1, G * NB + ROT)
            while st["pos"] < p1:
                g = st["pos"] // NB
                e = min(p1, (g + 1) * NB)
                score(g, st["pos"] - g * NB, e - g * NB)
                st["pos"] = e
                emit_pieces()

        for g in range(G):
            for j in range(NK):
                issue_to(g * NB + BOFF[j + 1] + LEAD)
                pv(g, j)
        issue_to(G * NB + ROT)
        assert st["nextp"] == len(ALLP)
        return st["bad"]

    bad = lax.fori_loop(0, NI, stage, jnp.zeros((1, TQ), f32))

    @pl.when(jnp.max(bad) > 0.0)
    def _():
        def unit(u, c):
            s = jnp.dot(kn_ref[:, 0:DH], qt_ref[u], preferred_element_type=f32)
            m = jnp.max(s, axis=0, keepdims=True)
            p = jnp.exp2(s - m)
            l = jnp.sum(p, axis=0, keepdims=True)
            o = jnp.dot(vt_ref[...].astype(bf16), p.astype(bf16), preferred_element_type=f32)
            ot_ref[u] = (o / l).astype(bf16)
            return c
        lax.fori_loop(0, NU, unit, 0)

    w_cp[5].wait()
    o_cp = [pltpu.make_async_copy(o_ref.at[pl.ds(a, b - a)], o_hbm.at[pl.ds(a, b - a)], sem_o.at[n])
            for n, (a, b) in enumerate(OSEG)]
    for n, (a, b) in enumerate(OSEG):
        t = a // TQ
        ot = ot_ref[t * H:(t + 1) * H, :, a - t * TQ:b - t * TQ].reshape(H * DH, b - a)
        att = lax.dot_general(ot, wo_ref[...], TN_DIMS, preferred_element_type=f32)
        o_ref[a:b, :] = (y_ref[a:b, :] + att).astype(bf16)
        o_cp[n].start()
    for c in o_cp:
        c.wait()


@jax.jit
def pallas_parallel_sum__grouped_kv_mqa__dense_activation_silu__prompt_kernel(
    A_x: jax.Array,
    A_wq: jax.Array,
    A_wk: jax.Array,
    A_wv: jax.Array,
    A_wo: jax.Array,
    B_x: jax.Array,
    B_w1: jax.Array,
    B_w2: jax.Array,
):
    del B_x
    anyspec = pl.BlockSpec(memory_space=pl.ANY)
    out = pl.pallas_call(
        _kernel,
        out_shape=jax.ShapeDtypeStruct((S, D), bf16),
        in_specs=[anyspec] * 7,
        out_specs=anyspec,
        scratch_shapes=[
            pltpu.VMEM((S, D), bf16),
            pltpu.VMEM((D, D), bf16),
            pltpu.VMEM((D + 2 * DH, D), bf16),
            pltpu.VMEM((D, D), bf16),
            pltpu.VMEM((F, D), bf16),
            pltpu.VMEM((F, D), bf16),
            pltpu.VMEM((S, D), bf16),
            pltpu.VMEM((S, D), bf16),
            pltpu.VMEM((NU, DH, TQ), bf16),
            pltpu.VMEM((NU, DH, TQ), f32),
            pltpu.VMEM((NU, TQ), f32),
            pltpu.VMEM((NI, G, TQ), f32),
            pltpu.VMEM((NB * 8, DE), u32),
            pltpu.VMEM((S, DE), bf16),
            pltpu.VMEM((NV, DE), bf16),
            pltpu.VMEM((DH, NV + NX, 128), f32),
            pltpu.VMEM((DH, S), f32),
            pltpu.VMEM((NU, DH, TQ), bf16),
            pltpu.VMEM((2, NV, TQ), f32),
            pltpu.VMEM((ROT * 16, TQ), f32),
            pltpu.VMEM((NU, NX, TQ), f32),
            pltpu.VMEM((S, D), f32),
            pltpu.VMEM((TQ, D), f32),
            pltpu.VMEM((TQ, F), bf16),
            pltpu.VMEM((DH, TQ), f32),
            pltpu.VMEM((8, 128), u32),
            pltpu.SemaphoreType.DMA((NT,)),
            pltpu.SemaphoreType.DMA((6,)),
            pltpu.SemaphoreType.DMA((len(OSEG),)),
        ],
        compiler_params=pltpu.CompilerParams(vmem_limit_bytes=100 * 1024 * 1024),
    )(A_x.reshape(S, D), A_wq, A_wk.T, A_wv.T, A_wo, B_w1.T, B_w2)
    return out.reshape(1, S, D)
```

```python
import math

import jax
import jax.numpy as jnp
import numpy as np
from jax import lax
import jax.experimental.pallas as pl
import jax.experimental.pallas.tpu as pltpu

S, D, H, DH, F = 2048, 512, 32, 16, 1376
TQ = 512
NT = S // TQ
NU = NT * H
KC = 128
NK = S // KC
NC = TQ // 128
DE = 32
QSCALE = (DH ** -0.5) * math.log2(math.e)
UP = 1.0 + 2.0 ** -6
L_MIN = 2.0 ** -60
EPS = 1e-5
f32, bf16, u32 = jnp.float32, jnp.bfloat16, jnp.uint32
NT_DIMS = (((1,), (1,)), ((), ()))
TN_DIMS = (((0,), (0,)), ((), ()))
FT = [(a, min(a + 128, F)) for a in range(0, F, 128)]

G = 8
NVL = [16, 16, 32, 16, 16, 16, 16, 32] + [16] * 8
NXL = [16, 0, 0, 0, 0] * 3 + [0]
LEAD = 8
ROT = 8
S1 = 8
HALF = 18
W1FRAC, F0, F1, FHALF = 0.5, 0.01, 0.03, 12
LN_AHEAD = 3
OSPLIT = 4


def _offsets(counts, div):
    return [int(v) // div for v in np.concatenate([[0], np.cumsum(counts)])]


GOFF, XOFF = _offsets(NVL, 8), _offsets(NXL, 8)
NV, NX = int(sum(NVL)), int(sum(NXL))
NBL = [(KC - v - w) // 16 for v, w in zip(NVL, NXL)]
BOFF = _offsets(NBL, 1)
NB = BOFF[-1]
NG, NGX = NV // 8, NX // 8
TILE_OF_GROUP = [j for j in range(NK) for _ in range(NVL[j] // 8)]
ALLP = [(g, r0 + r, c) for g in range(G) for r0 in range(0, NG, 2) for c in range(NC) for r in range(2)]
_LO, _HI = ROT * 8, (G * NB + ROT - S1) * 8
PTS = [min(_HI - 1, int(_LO + n * (_HI - _LO) / len(ALLP))) for n in range(len(ALLP))]
NI = NU // G
XP = [(h, r0 + r, c) for h in range(H) for r0 in range(0, NGX, 2) for c in range(NC) for r in range(2)]
XN1 = int(len(XP) * W1FRAC) // 2 * 2
XP1 = [int((F0 + (1 - F0) * n / XN1) * len(FT) * (TQ // 8)) for n in range(XN1)]
XP2 = [int((1 - F1) * n / (len(XP) - XN1) * len(FT) * (TQ // 8) * NC) for n in range(len(XP) - XN1)]
OSEG = ([(t * TQ, (t + 1) * TQ) for t in range(NT - 1)]
        + [((NT - 1) * TQ + k * (TQ // OSPLIT), (NT - 1) * TQ + (k + 1) * (TQ // OSPLIT)) for k in range(OSPLIT)])


def _kernel(x_hbm, wq_hbm, wkt_hbm, wvt_hbm, wo_hbm, w1t_hbm, w2_hbm, o_hbm,
            x_ref, wq_ref, wt_ref, wo_ref, w1t_ref, w2_ref, o_ref,
            xn_ref, qt_ref, qf_ref, nrm_ref, bias_ref, kx_ref, kn_ref, kv_ref, kb_ref,
            vt_ref, ot_ref, pvs_ref, pre_ref, px_ref, y_ref, ya_ref, h_ref, zf_ref, z_ref,
            sem_x, sem_w, sem_o):
    x_cp = [pltpu.make_async_copy(x_hbm.at[pl.ds(t * TQ, TQ)], x_ref.at[pl.ds(t * TQ, TQ)], sem_x.at[t])
            for t in range(NT)]
    w_cp = [pltpu.make_async_copy(a, b, sem_w.at[i]) for i, (a, b) in enumerate(
        [(wq_hbm, wq_ref), (wkt_hbm, wt_ref.at[pl.ds(D, DH)]), (wvt_hbm, wt_ref.at[pl.ds(D + DH, DH)]),
         (w1t_hbm, w1t_ref), (w2_hbm, w2_ref), (wo_hbm, wo_ref)])]
    for c in w_cp[:3]:
        c.start()
    x_cp[0].start()
    x_cp[1].start()
    zf_ref[...] = jnp.zeros(zf_ref.shape, f32)
    z_ref[...] = jnp.zeros(z_ref.shape, u32)

    row16 = lax.broadcasted_iota(jnp.int32, (DH, TQ), 0)
    row8 = lax.broadcasted_iota(jnp.int32, (8, TQ), 0)

    def layernorm(s, lk=None):
        x = x_ref[s * 128:(s + 1) * 128, :].astype(f32)
        if lk is not None:
            never = jnp.concatenate([z_ref[...] != 0] * 16, axis=0)
            x = jnp.concatenate([jnp.where(never, lk, x[:, 0:128]), x[:, 128:]], axis=1)
        mu = jnp.mean(x, axis=-1, keepdims=True)
        xc = x - mu
        var = jnp.mean(xc * xc, axis=-1, keepdims=True)
        xn_ref[s * 128:(s + 1) * 128, :] = (xc * lax.rsqrt(var + EPS)).astype(bf16)

    def proj_kv(t):
        xn = xn_ref[t * TQ:(t + 1) * TQ, :]
        r = lax.dot_general(wt_ref[D:D + 2 * DH, :], xn, NT_DIMS, preferred_element_type=f32)
        kt = r[0:DH].astype(bf16).astype(f32)
        vt_ref[:, t * TQ:(t + 1) * TQ] = r[DH:].astype(bf16).astype(f32)
        k2 = jnp.sum(kt * kt, axis=0, keepdims=True)
        ones_row = jnp.where(row16 == 0, 1.0, 0.0).astype(f32)
        ke = jnp.concatenate([kt, ones_row], axis=0).T
        kn_ref[t * TQ:(t + 1) * TQ, :] = ke.astype(bf16)
        for jj in range(TQ // KC):
            j = t * (TQ // KC) + jj
            for b in range(NBL[j]):
                src = jj * KC + NVL[j] + NXL[j] + 16 * (NBL[j] - 1 - b)
                kx_ref[8 * (BOFF[j] + b): 8 * (BOFF[j] + b) + 8, :] = pltpu.bitcast(
                    ke[src:src + 16, :].astype(bf16), u32)
            if NVL[j]:
                kv_ref[GOFF[j] * 8: GOFF[j] * 8 + NVL[j], :] = ke[jj * KC: jj * KC + NVL[j], :].astype(bf16)
            for r0 in range(0, NVL[j] + NXL[j], 8):
                kv = ke[jj * KC + r0: jj * KC + r0 + 8, :]
                dst = GOFF[j] * 8 + r0 if r0 < NVL[j] else NV + XOFF[j] * 8 + r0 - NVL[j]
                for d in range(DH):
                    kb_ref[d, dst:dst + 8, :] = jnp.broadcast_to(kv[:, d:d + 1], (8, 128))
        return k2

    def proj_q(s):
        t, a = s // NC, (s % NC) * 128
        xn = xn_ref[s * 128:(s + 1) * 128, :]
        r = lax.dot_general(wt_ref[0:D, :], xn, NT_DIMS, preferred_element_type=f32)
        qb = (r * QSCALE).astype(bf16)
        qf = qb.astype(f32).reshape(H, DH, 128)
        qt_ref[t * H:(t + 1) * H, :, a:a + 128] = qb.reshape(H, DH, 128)
        qf_ref[t * H:(t + 1) * H, :, a:a + 128] = qf
        nrm_ref[t * H:(t + 1) * H, a:a + 128] = jnp.sum(qf * qf, axis=1)
        return r

    def q_ext(it, g):
        brow = jnp.broadcast_to(bias_ref[it, g:g + 1, :], (8, TQ))
        blk = jnp.concatenate([jnp.where(row8 == 0, brow, 0.0), jnp.zeros((8, TQ), f32)], axis=0)
        return jnp.concatenate([qt_ref[G * it + g], blk.astype(bf16)], axis=0)

    for c in w_cp[:3]:
        c.wait()
    wt_ref[0:D, :] = wq_ref[...].T
    x_cp[0].wait()
    for c in x_cp[2:]:
        c.start()
    for s in range(NC):
        layernorm(s)
    for s in range(NC - 1):
        proj_q(s)
    for c in x_cp[1:]:
        c.wait()
    for c in w_cp[3:]:
        c.start()
    k2 = proj_kv(0)
    outs = {}
    nln = NC
    for s in range(NC - 1, NT * NC):
        while nln < NT * NC and nln - LN_AHEAD < s:
            lk = outs.get(nln - LN_AHEAD)
            if lk is not None:
                lk = jnp.concatenate([lk[32 * n:32 * n + 8] for n in range(16)], axis=0)
            layernorm(nln, lk)
            nln += 1
        if s % NC == NC - 1 and s >= NC:
            k2 = jnp.maximum(k2, proj_kv(s // NC))
        outs[s] = proj_q(s)
    kscale = jnp.sqrt(jnp.max(k2, axis=1, keepdims=True)) * (-UP)
    for t in range(NT):
        bias = (jnp.sqrt(nrm_ref[t * H:(t + 1) * H, :]) * kscale).astype(bf16).astype(f32)
        for k in range(H // G):
            bias_ref[t * (H // G) + k] = bias[k * G:(k + 1) * G]

    def vpu_probs(never, it, g, krow, c, lk, lk2=None):
        u = G * it + g
        acc = jnp.broadcast_to(bias_ref[it, g:g + 1, c * 128:(c + 1) * 128], (8, 128))
        acc = jnp.where(never, lk, acc)
        for d in range(DH):
            if d == DH // 2 and lk2 is not None:
                acc = jnp.where(never, lk2, acc)
            qb = jnp.broadcast_to(qf_ref[u, d:d + 1, c * 128:(c + 1) * 128], (8, 128))
            acc = acc + kb_ref[d, krow * 8:krow * 8 + 8, :] * qb
        return jnp.exp2(acc)

    def kblocks(b0, b1):
        return pltpu.bitcast(kx_ref[8 * b0:8 * b1, :], bf16)

    pvs_ref[0] = jnp.exp2(jnp.dot(kv_ref[...], q_ext(0, 0), preferred_element_type=f32))
    pre_ref[...] = jnp.exp2(jnp.dot(kblocks(0, ROT), q_ext(0, 0), preferred_element_type=f32))

    w_cp[3].wait()
    w_cp[4].wait()

    def ffn(t, carry):
        rows = pl.ds(pl.multiple_of(t * TQ, TQ), TQ)
        never = z_ref[...] != 0
        xn = xn_ref[rows, :]
        k = [0]

        parts = {}
        nv2 = TQ // 8 * NC

        def emit(lk, lk2=None):
            h, r, c = XP[k[0]]
            px_ref[t * H + h, r * 8:r * 8 + 8, c * 128:(c + 1) * 128] = vpu_probs(
                never, t * (H // G) + h // G, h % G, NG + r, c, lk, lk2)
            k[0] += 1

        def part_vreg(p):
            rg, cc = (p % nv2) // NC, p % NC
            return parts[p // nv2][rg * 8:rg * 8 + 8, cc * 128:(cc + 1) * 128]

        for n, (a, b) in enumerate(FT):
            h = lax.dot_general(xn, w1t_ref[a:b, :], NT_DIMS, preferred_element_type=f32)
            hh = h * 0.5
            h_ref[:, a:b] = (hh + hh * jnp.tanh(hh)).astype(bf16)
            while k[0] < XN1 and XP1[k[0]] // (TQ // 8) == n:
                rg = XP1[k[0]] % (TQ // 8)
                hv = h[rg * 8:rg * 8 + 8, :]
                if b - a < 128:
                    hv = jnp.concatenate([hv, hv[:, 0:128 - (b - a)]], axis=1)
                emit(hv)
        for n, (a, b) in enumerate(FT):
            part = jnp.dot(h_ref[:, a:b], w2_ref[a:b, :], preferred_element_type=f32)
            if n == 0:
                ya_ref[...] = x_ref[rows, :].astype(f32) + part
            elif n == len(FT) - 1:
                y_ref[rows, :] = ya_ref[...] + part
            else:
                ya_ref[...] += part
            parts[n] = part
            while k[0] < len(XP) and (XP2[k[0] - XN1] + FHALF) // nv2 <= n:
                p = XP2[k[0] - XN1]
                emit(part_vreg(p), part_vreg(p + FHALF))
        assert k[0] == len(XP)
        return carry

    lax.fori_loop(0, NT, ffn, 0)

    def stage(i, bad):
        L = [None] * G
        ACC = [None] * G
        Q = [None] * (G + 1)
        PM, SS = {}, {}
        done_v = set()
        st = dict(nextp=0, pos=ROT, bad=bad)
        never = z_ref[...] != 0
        inext = jnp.minimum(i + 1, NI - 1)

        def score_vreg(x):
            hf, cc = (x % 8) // 4, x % 4
            return SS[x // 8][8 * hf:8 * hf + 8, cc * 128:(cc + 1) * 128]

        def emit_pieces():
            while st["nextp"] < len(ALLP):
                g, r, c = ALLP[st["nextp"]]
                x = PTS[st["nextp"]]
                if ((x + HALF) // 8) not in SS or (g >= 1 and (g - 1, TILE_OF_GROUP[r]) not in done_v):
                    break
                it2, g2 = (i, g + 1) if g + 1 < G else (inext, 0)
                pvs_ref[g2 % 2, r * 8:r * 8 + 8, c * 128:(c + 1) * 128] = vpu_probs(
                    never, it2, g2, r, c, score_vreg(x), score_vreg(x + HALF))
                st["nextp"] += 1

        def score(g, b0, b1):
            if Q[g] is None:
                Q[g] = q_ext(i, g) if g < G else q_ext(inext, 0)
            s = jnp.dot(kblocks(b0, b1), Q[g], preferred_element_type=f32)
            p = jnp.exp2(s)
            if g == G:
                pre_ref[16 * b0:16 * b1, :] = p
            for b in range(b0, b1):
                PM[(g, b)] = p[16 * (b - b0):16 * (b - b0) + 16]
                SS[g * NB + b] = s[16 * (b - b0):16 * (b - b0) + 16]

        def pv(g, j):
            blocks = [(pre_ref[16 * b:16 * b + 16, :] if (g == 0 and b < ROT) else PM.pop((g, b)))
                      for b in range(BOFF[j], BOFF[j + 1])]
            if g >= 1:
                assert all((g - 1, r, c) in ALLP[:st["nextp"]]
                           for r in range(GOFF[j], GOFF[j + 1]) for c in range(NC))
            rows = [pvs_ref[g % 2, r * 8:r * 8 + 8, :] for r in range(GOFF[j], GOFF[j + 1])]
            rows += [px_ref[G * i + g, r * 8:r * 8 + 8, :] for r in range(XOFF[j], XOFF[j + 1])]
            for x in blocks:
                for y in (x[8:16], x[0:8]):
                    L[g] = y if L[g] is None else L[g] + y
            for x in reversed(rows):
                L[g] = L[g] + x
            pb = jnp.concatenate(rows + blocks[::-1], axis=0)
            o = jnp.dot(vt_ref[:, j * KC:(j + 1) * KC], pb, preferred_element_type=f32)
            if ACC[g] is None:
                ACC[g] = zf_ref[...]
            ACC[g] = ACC[g] + o
            if j == NK - 1:
                lsum = jnp.sum(L[g], axis=0, keepdims=True)
                ot_ref[G * i + g] = (ACC[g] / lsum).astype(bf16)
                st["bad"] = jnp.where(lsum >= L_MIN, st["bad"], 1.0)
            done_v.add((g, j))
            emit_pieces()

        def issue_to(p1):
            p1 = min(p1, G * NB + ROT)
            while st["pos"] < p1:
                g = st["pos"] // NB
                e = min(p1, (g + 1) * NB)
                score(g, st["pos"] - g * NB, e - g * NB)
                st["pos"] = e
                emit_pieces()

        for g in range(G):
            for j in range(NK):
                issue_to(g * NB + BOFF[j + 1] + LEAD)
                pv(g, j)
        issue_to(G * NB + ROT)
        assert st["nextp"] == len(ALLP)
        return st["bad"]

    bad = lax.fori_loop(0, NI, stage, jnp.zeros((1, TQ), f32))

    @pl.when(jnp.max(bad) > 0.0)
    def _():
        def unit(u, c):
            s = jnp.dot(kn_ref[:, 0:DH], qt_ref[u], preferred_element_type=f32)
            m = jnp.max(s, axis=0, keepdims=True)
            p = jnp.exp2(s - m)
            l = jnp.sum(p, axis=0, keepdims=True)
            o = jnp.dot(vt_ref[...].astype(bf16), p.astype(bf16), preferred_element_type=f32)
            ot_ref[u] = (o / l).astype(bf16)
            return c
        lax.fori_loop(0, NU, unit, 0)

    w_cp[5].wait()
    o_cp = [pltpu.make_async_copy(o_ref.at[pl.ds(a, b - a)], o_hbm.at[pl.ds(a, b - a)], sem_o.at[n])
            for n, (a, b) in enumerate(OSEG)]
    for n, (a, b) in enumerate(OSEG):
        t = a // TQ
        ot = ot_ref[t * H:(t + 1) * H, :, a - t * TQ:b - t * TQ].reshape(H * DH, b - a)
        att = lax.dot_general(ot, wo_ref[...], TN_DIMS, preferred_element_type=f32)
        o_ref[a:b, :] = (y_ref[a:b, :] + att).astype(bf16)
        o_cp[n].start()
    for c in o_cp:
        c.wait()


@jax.jit
def pallas_parallel_sum__grouped_kv_mqa__dense_activation_silu__prompt_kernel(
    A_x: jax.Array,
    A_wq: jax.Array,
    A_wk: jax.Array,
    A_wv: jax.Array,
    A_wo: jax.Array,
    B_x: jax.Array,
    B_w1: jax.Array,
    B_w2: jax.Array,
):
    del B_x
    anyspec = pl.BlockSpec(memory_space=pl.ANY)
    out = pl.pallas_call(
        _kernel,
        out_shape=jax.ShapeDtypeStruct((S, D), bf16),
        in_specs=[anyspec] * 7,
        out_specs=anyspec,
        scratch_shapes=[
            pltpu.VMEM((S, D), bf16),
            pltpu.VMEM((D, D), bf16),
            pltpu.VMEM((D + 2 * DH, D), bf16),
            pltpu.VMEM((D, D), bf16),
            pltpu.VMEM((F, D), bf16),
            pltpu.VMEM((F, D), bf16),
            pltpu.VMEM((S, D), bf16),
            pltpu.VMEM((S, D), bf16),
            pltpu.VMEM((NU, DH, TQ), bf16),
            pltpu.VMEM((NU, DH, TQ), f32),
            pltpu.VMEM((NU, TQ), f32),
            pltpu.VMEM((NI, G, TQ), f32),
            pltpu.VMEM((NB * 8, DE), u32),
            pltpu.VMEM((S, DE), bf16),
            pltpu.VMEM((NV, DE), bf16),
            pltpu.VMEM((DH, NV + NX, 128), f32),
            pltpu.VMEM((DH, S), f32),
            pltpu.VMEM((NU, DH, TQ), bf16),
            pltpu.VMEM((2, NV, TQ), f32),
            pltpu.VMEM((ROT * 16, TQ), f32),
            pltpu.VMEM((NU, NX, TQ), f32),
            pltpu.VMEM((S, D), f32),
            pltpu.VMEM((TQ, D), f32),
            pltpu.VMEM((TQ, F), bf16),
            pltpu.VMEM((DH, TQ), f32),
            pltpu.VMEM((8, 128), u32),
            pltpu.SemaphoreType.DMA((NT,)),
            pltpu.SemaphoreType.DMA((6,)),
            pltpu.SemaphoreType.DMA((len(OSEG),)),
        ],
        compiler_params=pltpu.CompilerParams(vmem_limit_bytes=100 * 1024 * 1024),
    )(A_x.reshape(S, D), A_wq, A_wk.T, A_wv.T, A_wo, B_w1.T, B_w2)
    return out.reshape(1, S, D)
```

```python
import math

import jax
import jax.numpy as jnp
import numpy as np
from jax import lax
import jax.experimental.pallas as pl
import jax.experimental.pallas.tpu as pltpu

S, D, H, DH, F = 2048, 512, 32, 16, 1376
TQ = 512
NT = S // TQ
NU = NT * H
KC = 128
NK = S // KC
NC = TQ // 128
DE = 32
QSCALE = (DH ** -0.5) * math.log2(math.e)
UP = 1.0 + 2.0 ** -6
L_MIN = 2.0 ** -60
EPS = 1e-5
f32, bf16, u32 = jnp.float32, jnp.bfloat16, jnp.uint32
NT_DIMS = (((1,), (1,)), ((), ()))
TN_DIMS = (((0,), (0,)), ((), ()))
FT = [(a, min(a + 128, F)) for a in range(0, F, 128)]

G = 8
NVL = [16, 16, 32, 16, 16, 16, 16, 32] + [16] * 8
NXL = [16, 0, 0, 0, 0] * 3 + [0]
LEAD = 8
ROT = 8
S1 = 8
HALF = 24
W1FRAC, F0, F1, FHALF = 0.5, 0.01, 0.03, 12
LN_AHEAD = 3
OSPLIT = 4


def _offsets(counts, div):
    return [int(v) // div for v in np.concatenate([[0], np.cumsum(counts)])]


GOFF, XOFF = _offsets(NVL, 8), _offsets(NXL, 8)
NV, NX = int(sum(NVL)), int(sum(NXL))
NBL = [(KC - v - w) // 16 for v, w in zip(NVL, NXL)]
BOFF = _offsets(NBL, 1)
NB = BOFF[-1]
NG, NGX = NV // 8, NX // 8
TILE_OF_GROUP = [j for j in range(NK) for _ in range(NVL[j] // 8)]
ALLP = [(g, r0 + r, c) for g in range(G) for r0 in range(0, NG, 2) for c in range(NC) for r in range(2)]
_LO, _HI = ROT * 8, (G * NB + ROT - S1) * 8
PTS = [min(_HI - 1, int(_LO + n * (_HI - _LO) / len(ALLP))) for n in range(len(ALLP))]
NI = NU // G
XP = [(h, r0 + r, c) for h in range(H) for r0 in range(0, NGX, 2) for c in range(NC) for r in range(2)]
XN1 = int(len(XP) * W1FRAC) // 2 * 2
XP1 = [int((F0 + (1 - F0) * n / XN1) * len(FT) * (TQ // 8)) for n in range(XN1)]
XP2 = [int((1 - F1) * n / (len(XP) - XN1) * len(FT) * (TQ // 8) * NC) for n in range(len(XP) - XN1)]
OSEG = ([(t * TQ, (t + 1) * TQ) for t in range(NT - 1)]
        + [((NT - 1) * TQ + k * (TQ // OSPLIT), (NT - 1) * TQ + (k + 1) * (TQ // OSPLIT)) for k in range(OSPLIT)])


def _kernel(x_hbm, wq_hbm, wkt_hbm, wvt_hbm, wo_hbm, w1t_hbm, w2_hbm, o_hbm,
            x_ref, wq_ref, wt_ref, wo_ref, w1t_ref, w2_ref, o_ref,
            xn_ref, qt_ref, qf_ref, nrm_ref, bias_ref, kx_ref, kn_ref, kv_ref, kb_ref,
            vt_ref, ot_ref, pvs_ref, pre_ref, px_ref, y_ref, ya_ref, h_ref, zf_ref, z_ref,
            sem_x, sem_w, sem_o):
    x_cp = [pltpu.make_async_copy(x_hbm.at[pl.ds(t * TQ, TQ)], x_ref.at[pl.ds(t * TQ, TQ)], sem_x.at[t])
            for t in range(NT)]
    w_cp = [pltpu.make_async_copy(a, b, sem_w.at[i]) for i, (a, b) in enumerate(
        [(wq_hbm, wq_ref), (wkt_hbm, wt_ref.at[pl.ds(D, DH)]), (wvt_hbm, wt_ref.at[pl.ds(D + DH, DH)]),
         (w1t_hbm, w1t_ref), (w2_hbm, w2_ref), (wo_hbm, wo_ref)])]
    for c in w_cp[:3]:
        c.start()
    x_cp[0].start()
    x_cp[1].start()
    zf_ref[...] = jnp.zeros(zf_ref.shape, f32)
    z_ref[...] = jnp.zeros(z_ref.shape, u32)

    row16 = lax.broadcasted_iota(jnp.int32, (DH, TQ), 0)
    row8 = lax.broadcasted_iota(jnp.int32, (8, TQ), 0)

    def layernorm(s, lk=None):
        x = x_ref[s * 128:(s + 1) * 128, :].astype(f32)
        if lk is not None:
            never = jnp.concatenate([z_ref[...] != 0] * 16, axis=0)
            x = jnp.concatenate([jnp.where(never, lk, x[:, 0:128]), x[:, 128:]], axis=1)
        mu = jnp.mean(x, axis=-1, keepdims=True)
        xc = x - mu
        var = jnp.mean(xc * xc, axis=-1, keepdims=True)
        xn_ref[s * 128:(s + 1) * 128, :] = (xc * lax.rsqrt(var + EPS)).astype(bf16)

    def proj_kv(t):
        xn = xn_ref[t * TQ:(t + 1) * TQ, :]
        r = lax.dot_general(wt_ref[D:D + 2 * DH, :], xn, NT_DIMS, preferred_element_type=f32)
        kt = r[0:DH].astype(bf16).astype(f32)
        vt_ref[:, t * TQ:(t + 1) * TQ] = r[DH:].astype(bf16).astype(f32)
        k2 = jnp.sum(kt * kt, axis=0, keepdims=True)
        ones_row = jnp.where(row16 == 0, 1.0, 0.0).astype(f32)
        ke = jnp.concatenate([kt, ones_row], axis=0).T
        kn_ref[t * TQ:(t + 1) * TQ, :] = ke.astype(bf16)
        for jj in range(TQ // KC):
            j = t * (TQ // KC) + jj
            for b in range(NBL[j]):
                src = jj * KC + NVL[j] + NXL[j] + 16 * (NBL[j] - 1 - b)
                kk = jnp.concatenate([ke[src + 8:src + 16, :], ke[src:src + 8, :]], axis=0)
                kx_ref[8 * (BOFF[j] + b): 8 * (BOFF[j] + b) + 8, :] = pltpu.bitcast(kk.astype(bf16), u32)
            if NVL[j]:
                kv_ref[GOFF[j] * 8: GOFF[j] * 8 + NVL[j], :] = ke[jj * KC: jj * KC + NVL[j], :].astype(bf16)
            for r0 in range(0, NVL[j] + NXL[j], 8):
                kv = ke[jj * KC + r0: jj * KC + r0 + 8, :]
                dst = GOFF[j] * 8 + r0 if r0 < NVL[j] else NV + XOFF[j] * 8 + r0 - NVL[j]
                for d in range(DH):
                    kb_ref[d, dst:dst + 8, :] = jnp.broadcast_to(kv[:, d:d + 1], (8, 128))
        return k2

    def proj_q(s):
        t, a = s // NC, (s % NC) * 128
        xn = xn_ref[s * 128:(s + 1) * 128, :]
        r = lax.dot_general(wt_ref[0:D, :], xn, NT_DIMS, preferred_element_type=f32)
        qb = (r * QSCALE).astype(bf16)
        qf = qb.astype(f32).reshape(H, DH, 128)
        qt_ref[t * H:(t + 1) * H, :, a:a + 128] = qb.reshape(H, DH, 128)
        qf_ref[t * H:(t + 1) * H, :, a:a + 128] = qf
        nrm_ref[t * H:(t + 1) * H, a:a + 128] = jnp.sum(qf * qf, axis=1)
        return r

    def q_ext(it, g):
        brow = jnp.broadcast_to(bias_ref[it, g:g + 1, :], (8, TQ))
        blk = jnp.concatenate([jnp.where(row8 == 0, brow, 0.0), jnp.zeros((8, TQ), f32)], axis=0)
        return jnp.concatenate([qt_ref[G * it + g], blk.astype(bf16)], axis=0)

    for c in w_cp[:3]:
        c.wait()
    wt_ref[0:D, :] = wq_ref[...].T
    x_cp[0].wait()
    for c in x_cp[2:]:
        c.start()
    for s in range(NC):
        layernorm(s)
    for s in range(NC - 1):
        proj_q(s)
    for c in x_cp[1:]:
        c.wait()
    for c in w_cp[3:]:
        c.start()
    k2 = proj_kv(0)
    outs = {}
    nln = NC
    for s in range(NC - 1, NT * NC):
        while nln < NT * NC and nln - LN_AHEAD < s:
            lk = outs.get(nln - LN_AHEAD)
            if lk is not None:
                lk = jnp.concatenate([lk[32 * n:32 * n + 8] for n in range(16)], axis=0)
            layernorm(nln, lk)
            nln += 1
        if s % NC == NC - 1 and s >= NC:
            k2 = jnp.maximum(k2, proj_kv(s // NC))
        outs[s] = proj_q(s)
    kscale = jnp.sqrt(jnp.max(k2, axis=1, keepdims=True)) * (-UP)
    for t in range(NT):
        bias = (jnp.sqrt(nrm_ref[t * H:(t + 1) * H, :]) * kscale).astype(bf16).astype(f32)
        for k in range(H // G):
            bias_ref[t * (H // G) + k] = bias[k * G:(k + 1) * G]

    def vpu_probs(never, it, g, krow, c, lk, lk2=None):
        u = G * it + g
        acc = jnp.broadcast_to(bias_ref[it, g:g + 1, c * 128:(c + 1) * 128], (8, 128))
        acc = jnp.where(never, lk, acc)
        for d in range(DH):
            if d == DH // 2 and lk2 is not None:
                acc = jnp.where(never, lk2, acc)
            qb = jnp.broadcast_to(qf_ref[u, d:d + 1, c * 128:(c + 1) * 128], (8, 128))
            acc = acc + kb_ref[d, krow * 8:krow * 8 + 8, :] * qb
        return jnp.exp2(acc)

    def kblocks(b0, b1):
        return pltpu.bitcast(kx_ref[8 * b0:8 * b1, :], bf16)

    pvs_ref[0] = jnp.exp2(jnp.dot(kv_ref[...], q_ext(0, 0), preferred_element_type=f32))
    pre_ref[...] = jnp.exp2(jnp.dot(kblocks(0, ROT), q_ext(0, 0), preferred_element_type=f32))

    w_cp[3].wait()
    w_cp[4].wait()

    def ffn(t, carry):
        rows = pl.ds(pl.multiple_of(t * TQ, TQ), TQ)
        never = z_ref[...] != 0
        xn = xn_ref[rows, :]
        k = [0]

        parts = {}
        nv2 = TQ // 8 * NC

        def emit(lk, lk2=None):
            h, r, c = XP[k[0]]
            px_ref[t * H + h, r * 8:r * 8 + 8, c * 128:(c + 1) * 128] = vpu_probs(
                never, t * (H // G) + h // G, h % G, NG + r, c, lk, lk2)
            k[0] += 1

        def part_vreg(p):
            rg, cc = (p % nv2) // NC, p % NC
            return parts[p // nv2][rg * 8:rg * 8 + 8, cc * 128:(cc + 1) * 128]

        for n, (a, b) in enumerate(FT):
            h = lax.dot_general(xn, w1t_ref[a:b, :], NT_DIMS, preferred_element_type=f32)
            hh = h * 0.5
            h_ref[:, a:b] = (hh + hh * jnp.tanh(hh)).astype(bf16)
            while k[0] < XN1 and XP1[k[0]] // (TQ // 8) == n:
                rg = XP1[k[0]] % (TQ // 8)
                hv = h[rg * 8:rg * 8 + 8, :]
                if b - a < 128:
                    hv = jnp.concatenate([hv, hv[:, 0:128 - (b - a)]], axis=1)
                emit(hv)
        for n, (a, b) in enumerate(FT):
            part = jnp.dot(h_ref[:, a:b], w2_ref[a:b, :], preferred_element_type=f32)
            if n == 0:
                ya_ref[...] = x_ref[rows, :].astype(f32) + part
            elif n == len(FT) - 1:
                y_ref[rows, :] = ya_ref[...] + part
            else:
                ya_ref[...] += part
            parts[n] = part
            while k[0] < len(XP) and (XP2[k[0] - XN1] + FHALF) // nv2 <= n:
                p = XP2[k[0] - XN1]
                emit(part_vreg(p), part_vreg(p + FHALF))
        assert k[0] == len(XP)
        return carry

    lax.fori_loop(0, NT, ffn, 0)

    def stage(i, bad):
        L = [None] * G
        ACC = [None] * G
        Q = [None] * (G + 1)
        PM, SS = {}, {}
        done_v = set()
        st = dict(nextp=0, pos=ROT, bad=bad)
        never = z_ref[...] != 0
        inext = jnp.minimum(i + 1, NI - 1)

        def score_vreg(x):
            hf, cc = (x % 8) // 4, x % 4
            return SS[x // 8][8 * hf:8 * hf + 8, cc * 128:(cc + 1) * 128]

        def emit_pieces():
            while st["nextp"] < len(ALLP):
                g, r, c = ALLP[st["nextp"]]
                x = PTS[st["nextp"]]
                if ((x + HALF) // 8) not in SS or (g >= 1 and (g - 1, TILE_OF_GROUP[r]) not in done_v):
                    break
                it2, g2 = (i, g + 1) if g + 1 < G else (inext, 0)
                pvs_ref[g2 % 2, r * 8:r * 8 + 8, c * 128:(c + 1) * 128] = vpu_probs(
                    never, it2, g2, r, c, score_vreg(x), score_vreg(x + HALF))
                st["nextp"] += 1

        def score(g, b0, b1):
            if Q[g] is None:
                Q[g] = q_ext(i, g) if g < G else q_ext(inext, 0)
            s = jnp.dot(kblocks(b0, b1), Q[g], preferred_element_type=f32)
            p = jnp.exp2(s)
            if g == G:
                pre_ref[16 * b0:16 * b1, :] = p
            for b in range(b0, b1):
                PM[(g, b)] = p[16 * (b - b0):16 * (b - b0) + 16]
                SS[g * NB + b] = s[16 * (b - b0):16 * (b - b0) + 16]

        def pv(g, j):
            blocks = [(pre_ref[16 * b:16 * b + 16, :] if (g == 0 and b < ROT) else PM.pop((g, b)))
                      for b in range(BOFF[j], BOFF[j + 1])]
            blocks = [y for x in blocks for y in (x[0:8], x[8:16])]
            if g >= 1:
                assert all((g - 1, r, c) in ALLP[:st["nextp"]]
                           for r in range(GOFF[j], GOFF[j + 1]) for c in range(NC))
            rows = [pvs_ref[g % 2, r * 8:r * 8 + 8, :] for r in range(GOFF[j], GOFF[j + 1])]
            rows += [px_ref[G * i + g, r * 8:r * 8 + 8, :] for r in range(XOFF[j], XOFF[j + 1])]
            for x in blocks + rows[::-1]:
                L[g] = x if L[g] is None else L[g] + x
            pb = jnp.concatenate(rows + blocks[::-1], axis=0)
            o = jnp.dot(vt_ref[:, j * KC:(j + 1) * KC], pb, preferred_element_type=f32)
            if ACC[g] is None:
                ACC[g] = zf_ref[...]
            ACC[g] = ACC[g] + o
            if j == NK - 1:
                lsum = jnp.sum(L[g], axis=0, keepdims=True)
                ot_ref[G * i + g] = (ACC[g] / lsum).astype(bf16)
                st["bad"] = jnp.where(lsum >= L_MIN, st["bad"], 1.0)
            done_v.add((g, j))
            emit_pieces()

        def issue_to(p1):
            p1 = min(p1, G * NB + ROT)
            while st["pos"] < p1:
                g = st["pos"] // NB
                e = min(p1, (g + 1) * NB)
                score(g, st["pos"] - g * NB, e - g * NB)
                st["pos"] = e
                emit_pieces()

        for g in range(G):
            for j in range(NK):
                issue_to(g * NB + BOFF[j + 1] + LEAD)
                pv(g, j)
        issue_to(G * NB + ROT)
        assert st["nextp"] == len(ALLP)
        return st["bad"]

    bad = lax.fori_loop(0, NI, stage, jnp.zeros((1, TQ), f32))

    @pl.when(jnp.max(bad) > 0.0)
    def _():
        def unit(u, c):
            s = jnp.dot(kn_ref[:, 0:DH], qt_ref[u], preferred_element_type=f32)
            m = jnp.max(s, axis=0, keepdims=True)
            p = jnp.exp2(s - m)
            l = jnp.sum(p, axis=0, keepdims=True)
            o = jnp.dot(vt_ref[...].astype(bf16), p.astype(bf16), preferred_element_type=f32)
            ot_ref[u] = (o / l).astype(bf16)
            return c
        lax.fori_loop(0, NU, unit, 0)

    w_cp[5].wait()
    o_cp = [pltpu.make_async_copy(o_ref.at[pl.ds(a, b - a)], o_hbm.at[pl.ds(a, b - a)], sem_o.at[n])
            for n, (a, b) in enumerate(OSEG)]
    for n, (a, b) in enumerate(OSEG):
        t = a // TQ
        ot = ot_ref[t * H:(t + 1) * H, :, a - t * TQ:b - t * TQ].reshape(H * DH, b - a)
        att = lax.dot_general(ot, wo_ref[...], TN_DIMS, preferred_element_type=f32)
        o_ref[a:b, :] = (y_ref[a:b, :] + att).astype(bf16)
        o_cp[n].start()
    for c in o_cp:
        c.wait()


@jax.jit
def pallas_parallel_sum__grouped_kv_mqa__dense_activation_silu__prompt_kernel(
    A_x: jax.Array,
    A_wq: jax.Array,
    A_wk: jax.Array,
    A_wv: jax.Array,
    A_wo: jax.Array,
    B_x: jax.Array,
    B_w1: jax.Array,
    B_w2: jax.Array,
):
    del B_x
    anyspec = pl.BlockSpec(memory_space=pl.ANY)
    out = pl.pallas_call(
        _kernel,
        out_shape=jax.ShapeDtypeStruct((S, D), bf16),
        in_specs=[anyspec] * 7,
        out_specs=anyspec,
        scratch_shapes=[
            pltpu.VMEM((S, D), bf16),
            pltpu.VMEM((D, D), bf16),
            pltpu.VMEM((D + 2 * DH, D), bf16),
            pltpu.VMEM((D, D), bf16),
            pltpu.VMEM((F, D), bf16),
            pltpu.VMEM((F, D), bf16),
            pltpu.VMEM((S, D), bf16),
            pltpu.VMEM((S, D), bf16),
            pltpu.VMEM((NU, DH, TQ), bf16),
            pltpu.VMEM((NU, DH, TQ), f32),
            pltpu.VMEM((NU, TQ), f32),
            pltpu.VMEM((NI, G, TQ), f32),
            pltpu.VMEM((NB * 8, DE), u32),
            pltpu.VMEM((S, DE), bf16),
            pltpu.VMEM((NV, DE), bf16),
            pltpu.VMEM((DH, NV + NX, 128), f32),
            pltpu.VMEM((DH, S), f32),
            pltpu.VMEM((NU, DH, TQ), bf16),
            pltpu.VMEM((2, NV, TQ), f32),
            pltpu.VMEM((ROT * 16, TQ), f32),
            pltpu.VMEM((NU, NX, TQ), f32),
            pltpu.VMEM((S, D), f32),
            pltpu.VMEM((TQ, D), f32),
            pltpu.VMEM((TQ, F), bf16),
            pltpu.VMEM((DH, TQ), f32),
            pltpu.VMEM((8, 128), u32),
            pltpu.SemaphoreType.DMA((NT,)),
            pltpu.SemaphoreType.DMA((6,)),
            pltpu.SemaphoreType.DMA((len(OSEG),)),
        ],
        compiler_params=pltpu.CompilerParams(vmem_limit_bytes=100 * 1024 * 1024),
    )(A_x.reshape(S, D), A_wq, A_wk.T, A_wv.T, A_wo, B_w1.T, B_w2)
    return out.reshape(1, S, D)
```

```python
import math

import jax
import jax.numpy as jnp
import numpy as np
from jax import lax
import jax.experimental.pallas as pl
import jax.experimental.pallas.tpu as pltpu

S, D, H, DH, F = 2048, 512, 32, 16, 1376
TQ = 512
NT = S // TQ
NU = NT * H
KC = 128
NK = S // KC
NC = TQ // 128
DE = 32
QSCALE = (DH ** -0.5) * math.log2(math.e)
UP = 1.0 + 2.0 ** -6
L_MIN = 2.0 ** -60
EPS = 1e-5
f32, bf16, u32 = jnp.float32, jnp.bfloat16, jnp.uint32
NT_DIMS = (((1,), (1,)), ((), ()))
TN_DIMS = (((0,), (0,)), ((), ()))
FT = [(a, min(a + 128, F)) for a in range(0, F, 128)]

G = 8
NVL = [16, 16, 32, 16, 16, 16, 16, 32] + [16] * 8
NXL = [16, 0, 0, 0, 0] * 3 + [0]
LEAD = 8
ROT = 8
S1 = 8
HALF = 24
W1FRAC, F0, F1, FHALF = 0.5, 0.01, 0.03, 12
LN_AHEAD = 3
OSPLIT = 4


def _offsets(counts, div):
    return [int(v) // div for v in np.concatenate([[0], np.cumsum(counts)])]


GOFF, XOFF = _offsets(NVL, 8), _offsets(NXL, 8)
NV, NX = int(sum(NVL)), int(sum(NXL))
NBL = [(KC - v - w) // 16 for v, w in zip(NVL, NXL)]
BOFF = _offsets(NBL, 1)
NB = BOFF[-1]
NG, NGX = NV // 8, NX // 8
TILE_OF_GROUP = [j for j in range(NK) for _ in range(NVL[j] // 8)]
ALLP = [(g, r0 + r, c) for g in range(G) for r0 in range(0, NG, 2) for c in range(NC) for r in range(2)]
_LO, _HI = ROT * 8, (G * NB + ROT - S1) * 8
PTS = [min(_HI - 1, int(_LO + n * (_HI - _LO) / len(ALLP))) for n in range(len(ALLP))]
NI = NU // G
XP = [(h, r0 + r, c) for h in range(H) for r0 in range(0, NGX, 2) for c in range(NC) for r in range(2)]
XN1 = int(len(XP) * W1FRAC) // 2 * 2
XP1 = [int((F0 + (1 - F0) * n / XN1) * len(FT) * (TQ // 8)) for n in range(XN1)]
XP2 = [int((1 - F1) * n / (len(XP) - XN1) * len(FT) * (TQ // 8) * NC) for n in range(len(XP) - XN1)]
OSEG = ([(t * TQ, (t + 1) * TQ) for t in range(NT - 1)]
        + [((NT - 1) * TQ + k * (TQ // OSPLIT), (NT - 1) * TQ + (k + 1) * (TQ // OSPLIT)) for k in range(OSPLIT)])


def _kernel(x_hbm, wq_hbm, wkt_hbm, wvt_hbm, wo_hbm, w1t_hbm, w2_hbm, o_hbm,
            x_ref, wq_ref, wt_ref, wo_ref, w1t_ref, w2_ref, o_ref,
            xn_ref, qt_ref, qf_ref, nrm_ref, bias_ref, kx_ref, kn_ref, kv_ref, kb_ref,
            vt_ref, ot_ref, pvs_ref, pre_ref, px_ref, y_ref, ya_ref, h_ref, zf_ref, z_ref,
            sem_x, sem_w, sem_o):
    x_cp = [pltpu.make_async_copy(x_hbm.at[pl.ds(t * TQ, TQ)], x_ref.at[pl.ds(t * TQ, TQ)], sem_x.at[t])
            for t in range(NT)]
    w_cp = [pltpu.make_async_copy(a, b, sem_w.at[i]) for i, (a, b) in enumerate(
        [(wq_hbm, wq_ref), (wkt_hbm, wt_ref.at[pl.ds(D, DH)]), (wvt_hbm, wt_ref.at[pl.ds(D + DH, DH)]),
         (w1t_hbm, w1t_ref), (w2_hbm, w2_ref), (wo_hbm, wo_ref)])]
    for c in w_cp[:3]:
        c.start()
    x_cp[0].start()
    x_cp[1].start()
    zf_ref[...] = jnp.zeros(zf_ref.shape, f32)
    z_ref[...] = jnp.zeros(z_ref.shape, u32)

    row16 = lax.broadcasted_iota(jnp.int32, (DH, TQ), 0)
    row8 = lax.broadcasted_iota(jnp.int32, (8, TQ), 0)

    def layernorm(s, lk=None):
        x = x_ref[s * 128:(s + 1) * 128, :].astype(f32)
        if lk is not None:
            never = jnp.concatenate([z_ref[...] != 0] * 16, axis=0)
            x = jnp.concatenate([jnp.where(never, lk, x[:, 0:128]), x[:, 128:]], axis=1)
        mu = jnp.mean(x, axis=-1, keepdims=True)
        xc = x - mu
        var = jnp.mean(xc * xc, axis=-1, keepdims=True)
        xn_ref[s * 128:(s + 1) * 128, :] = (xc * lax.rsqrt(var + EPS)).astype(bf16)

    def proj_kv(t):
        xn = xn_ref[t * TQ:(t + 1) * TQ, :]
        r = lax.dot_general(wt_ref[D:D + 2 * DH, :], xn, NT_DIMS, preferred_element_type=f32)
        kt = r[0:DH].astype(bf16).astype(f32)
        vt_ref[:, t * TQ:(t + 1) * TQ] = r[DH:].astype(bf16).astype(f32)
        k2 = jnp.sum(kt * kt, axis=0, keepdims=True)
        ones_row = jnp.where(row16 == 0, 1.0, 0.0).astype(f32)
        ke = jnp.concatenate([kt, ones_row], axis=0).T
        kn_ref[t * TQ:(t + 1) * TQ, :] = ke.astype(bf16)
        for jj in range(TQ // KC):
            j = t * (TQ // KC) + jj
            for b in range(NBL[j]):
                src = jj * KC + NVL[j] + NXL[j] + 16 * (NBL[j] - 1 - b)
                kk = jnp.concatenate([ke[src + 8:src + 16, :], ke[src:src + 8, :]], axis=0)
                kx_ref[8 * (BOFF[j] + b): 8 * (BOFF[j] + b) + 8, :] = pltpu.bitcast(kk.astype(bf16), u32)
            if NVL[j]:
                kv_ref[GOFF[j] * 8: GOFF[j] * 8 + NVL[j], :] = ke[jj * KC: jj * KC + NVL[j], :].astype(bf16)
            for r0 in range(0, NVL[j] + NXL[j], 8):
                kv = ke[jj * KC + r0: jj * KC + r0 + 8, :]
                dst = GOFF[j] * 8 + r0 if r0 < NVL[j] else NV + XOFF[j] * 8 + r0 - NVL[j]
                for d in range(DH):
                    kb_ref[d, dst:dst + 8, :] = jnp.broadcast_to(kv[:, d:d + 1], (8, 128))
        return k2

    def proj_q(s):
        t, a = s // NC, (s % NC) * 128
        xn = xn_ref[s * 128:(s + 1) * 128, :]
        r = lax.dot_general(wt_ref[0:D, :], xn, NT_DIMS, preferred_element_type=f32)
        qb = (r * QSCALE).astype(bf16)
        qf = qb.astype(f32).reshape(H, DH, 128)
        qt_ref[t * H:(t + 1) * H, :, a:a + 128] = qb.reshape(H, DH, 128)
        qf_ref[t * H:(t + 1) * H, :, a:a + 128] = qf
        nrm_ref[t * H:(t + 1) * H, a:a + 128] = jnp.sum(qf * qf, axis=1)
        return r

    def q_ext(it, g):
        brow = jnp.broadcast_to(bias_ref[it, g:g + 1, :], (8, TQ))
        blk = jnp.concatenate([jnp.where(row8 == 0, brow, 0.0), jnp.zeros((8, TQ), f32)], axis=0)
        return jnp.concatenate([qt_ref[G * it + g], blk.astype(bf16)], axis=0)

    for c in w_cp[:3]:
        c.wait()
    wt_ref[0:D, :] = wq_ref[...].T
    x_cp[0].wait()
    for c in x_cp[2:]:
        c.start()
    for s in range(NC):
        layernorm(s)
    for s in range(NC - 1):
        proj_q(s)
    for c in x_cp[1:]:
        c.wait()
    for c in w_cp[3:]:
        c.start()
    k2 = proj_kv(0)
    outs = {}
    nln = NC
    for s in range(NC - 1, NT * NC):
        while nln < NT * NC and nln - LN_AHEAD < s:
            lk = outs.get(nln - LN_AHEAD)
            if lk is not None:
                lk = jnp.concatenate([lk[32 * n:32 * n + 8] for n in range(16)], axis=0)
            layernorm(nln, lk)
            nln += 1
        if s % NC == NC - 1 and s >= NC:
            k2 = jnp.maximum(k2, proj_kv(s // NC))
        outs[s] = proj_q(s)
    kscale = jnp.sqrt(jnp.max(k2, axis=1, keepdims=True)) * (-UP)
    for t in range(NT):
        bias = (jnp.sqrt(nrm_ref[t * H:(t + 1) * H, :]) * kscale).astype(bf16).astype(f32)
        for k in range(H // G):
            bias_ref[t * (H // G) + k] = bias[k * G:(k + 1) * G]

    def vpu_probs(never, it, g, krow, c, lk, lk2=None):
        u = G * it + g
        acc = jnp.broadcast_to(bias_ref[it, g:g + 1, c * 128:(c + 1) * 128], (16, 128))
        acc = jnp.where(never, jnp.concatenate(lk, axis=0), acc)
        for d in range(DH):
            if d == DH // 2 and lk2 is not None:
                acc = jnp.where(never, jnp.concatenate(lk2, axis=0), acc)
            qb = jnp.broadcast_to(qf_ref[u, d:d + 1, c * 128:(c + 1) * 128], (16, 128))
            acc = acc + kb_ref[d, krow * 8:krow * 8 + 16, :] * qb
        return jnp.exp2(acc)

    def kblocks(b0, b1):
        return pltpu.bitcast(kx_ref[8 * b0:8 * b1, :], bf16)

    pvs_ref[0] = jnp.exp2(jnp.dot(kv_ref[...], q_ext(0, 0), preferred_element_type=f32))
    pre_ref[...] = jnp.exp2(jnp.dot(kblocks(0, ROT), q_ext(0, 0), preferred_element_type=f32))

    w_cp[3].wait()
    w_cp[4].wait()

    def ffn(t, carry):
        rows = pl.ds(pl.multiple_of(t * TQ, TQ), TQ)
        never = jnp.concatenate([z_ref[...] != 0] * 2, axis=0)
        xn = xn_ref[rows, :]
        k = [0]

        hs, parts = {}, {}
        nv1, nv2 = TQ // 8, TQ // 8 * NC

        def emit(lk, lk2=None):
            h, r, c = XP[k[0]]
            assert XP[k[0] + 1] == (h, r + 1, c)
            px_ref[t * H + h, r * 8:r * 8 + 16, c * 128:(c + 1) * 128] = vpu_probs(
                never, t * (H // G) + h // G, h % G, NG + r, c, lk, lk2)
            k[0] += 2

        def h_vreg(p):
            hv = hs[p // nv1][(p % nv1) * 8:(p % nv1) * 8 + 8, :]
            if hv.shape[1] < 128:
                hv = jnp.concatenate([hv, hv[:, 0:128 - hv.shape[1]]], axis=1)
            return hv

        def part_vreg(p):
            rg, cc = (p % nv2) // NC, p % NC
            return parts[p // nv2][rg * 8:rg * 8 + 8, cc * 128:(cc + 1) * 128]

        for n, (a, b) in enumerate(FT):
            h = lax.dot_general(xn, w1t_ref[a:b, :], NT_DIMS, preferred_element_type=f32)
            hh = h * 0.5
            h_ref[:, a:b] = (hh + hh * jnp.tanh(hh)).astype(bf16)
            hs[n] = h
            while k[0] < XN1 and XP1[k[0] + 1] // nv1 <= n:
                emit([h_vreg(p) for p in XP1[k[0]:k[0] + 2]])
        for n, (a, b) in enumerate(FT):
            part = jnp.dot(h_ref[:, a:b], w2_ref[a:b, :], preferred_element_type=f32)
            if n == 0:
                ya_ref[...] = x_ref[rows, :].astype(f32) + part
            elif n == len(FT) - 1:
                y_ref[rows, :] = ya_ref[...] + part
            else:
                ya_ref[...] += part
            parts[n] = part
            while k[0] < len(XP) and (XP2[k[0] + 1 - XN1] + FHALF) // nv2 <= n:
                ps = XP2[k[0] - XN1:k[0] - XN1 + 2]
                emit([part_vreg(p) for p in ps], [part_vreg(p + FHALF) for p in ps])
        assert k[0] == len(XP)
        return carry

    lax.fori_loop(0, NT, ffn, 0)

    def stage(i, bad):
        L = [None] * G
        ACC = [None] * G
        Q = [None] * (G + 1)
        PM, SS = {}, {}
        done_v = set()
        st = dict(nextp=0, pos=ROT, bad=bad)
        never = jnp.concatenate([z_ref[...] != 0] * 2, axis=0)
        inext = jnp.minimum(i + 1, NI - 1)

        def score_vreg(x):
            hf, cc = (x % 8) // 4, x % 4
            return SS[x // 8][8 * hf:8 * hf + 8, cc * 128:(cc + 1) * 128]

        def emit_pieces():
            while st["nextp"] < len(ALLP):
                g, r, c = ALLP[st["nextp"]]
                xs = PTS[st["nextp"]:st["nextp"] + 2]
                if ((xs[1] + HALF) // 8) not in SS or (g >= 1 and (g - 1, TILE_OF_GROUP[r + 1]) not in done_v):
                    break
                it2, g2 = (i, g + 1) if g + 1 < G else (inext, 0)
                pvs_ref[g2 % 2, r * 8:r * 8 + 16, c * 128:(c + 1) * 128] = vpu_probs(
                    never, it2, g2, r, c, [score_vreg(x) for x in xs], [score_vreg(x + HALF) for x in xs])
                st["nextp"] += 2

        def score(g, b0, b1):
            if Q[g] is None:
                Q[g] = q_ext(i, g) if g < G else q_ext(inext, 0)
            s = jnp.dot(kblocks(b0, b1), Q[g], preferred_element_type=f32)
            p = jnp.exp2(s)
            if g == G:
                pre_ref[16 * b0:16 * b1, :] = p
            for b in range(b0, b1):
                PM[(g, b)] = p[16 * (b - b0):16 * (b - b0) + 16]
                SS[g * NB + b] = s[16 * (b - b0):16 * (b - b0) + 16]

        def pv(g, j):
            blocks = [(pre_ref[16 * b:16 * b + 16, :] if (g == 0 and b < ROT) else PM.pop((g, b)))
                      for b in range(BOFF[j], BOFF[j + 1])]
            blocks = [y for x in blocks for y in (x[0:8], x[8:16])]
            if g >= 1:
                assert all((g - 1, r, c) in ALLP[:st["nextp"]]
                           for r in range(GOFF[j], GOFF[j + 1]) for c in range(NC))
            rows = [pvs_ref[g % 2, r * 8:r * 8 + 8, :] for r in range(GOFF[j], GOFF[j + 1])]
            rows += [px_ref[G * i + g, r * 8:r * 8 + 8, :] for r in range(XOFF[j], XOFF[j + 1])]
            for x in blocks + rows[::-1]:
                L[g] = x if L[g] is None else L[g] + x
            pb = jnp.concatenate(rows + blocks[::-1], axis=0)
            o = jnp.dot(vt_ref[:, j * KC:(j + 1) * KC], pb, preferred_element_type=f32,
                        precision=lax.Precision.DEFAULT)
            if ACC[g] is None:
                ACC[g] = zf_ref[...]
            ACC[g] = ACC[g] + o
            if j == NK - 1:
                lsum = jnp.sum(L[g], axis=0, keepdims=True)
                ot_ref[G * i + g] = (ACC[g] / lsum).astype(bf16)
                st["bad"] = jnp.where(lsum >= L_MIN, st["bad"], 1.0)
            done_v.add((g, j))
            emit_pieces()

        def issue_to(p1):
            p1 = min(p1, G * NB + ROT)
            while st["pos"] < p1:
                g = st["pos"] // NB
                e = min(p1, (g + 1) * NB)
                score(g, st["pos"] - g * NB, e - g * NB)
                st["pos"] = e
                emit_pieces()

        for g in range(G):
            for j in range(NK):
                issue_to(g * NB + BOFF[j + 1] + LEAD)
                pv(g, j)
        issue_to(G * NB + ROT)
        assert st["nextp"] == len(ALLP)
        return st["bad"]

    bad = lax.fori_loop(0, NI, stage, jnp.zeros((1, TQ), f32))

    @pl.when(jnp.max(bad) > 0.0)
    def _():
        def unit(u, c):
            s = jnp.dot(kn_ref[:, 0:DH], qt_ref[u], preferred_element_type=f32)
            m = jnp.max(s, axis=0, keepdims=True)
            p = jnp.exp2(s - m)
            l = jnp.sum(p, axis=0, keepdims=True)
            o = jnp.dot(vt_ref[...].astype(bf16), p.astype(bf16), preferred_element_type=f32)
            ot_ref[u] = (o / l).astype(bf16)
            return c
        lax.fori_loop(0, NU, unit, 0)

    w_cp[5].wait()
    o_cp = [pltpu.make_async_copy(o_ref.at[pl.ds(a, b - a)], o_hbm.at[pl.ds(a, b - a)], sem_o.at[n])
            for n, (a, b) in enumerate(OSEG)]
    for n, (a, b) in enumerate(OSEG):
        t = a // TQ
        ot = ot_ref[t * H:(t + 1) * H, :, a - t * TQ:b - t * TQ].reshape(H * DH, b - a)
        att = lax.dot_general(ot, wo_ref[...], TN_DIMS, preferred_element_type=f32)
        o_ref[a:b, :] = (y_ref[a:b, :] + att).astype(bf16)
        o_cp[n].start()
    for c in o_cp:
        c.wait()


@jax.jit
def pallas_parallel_sum__grouped_kv_mqa__dense_activation_silu__prompt_kernel(
    A_x: jax.Array,
    A_wq: jax.Array,
    A_wk: jax.Array,
    A_wv: jax.Array,
    A_wo: jax.Array,
    B_x: jax.Array,
    B_w1: jax.Array,
    B_w2: jax.Array,
):
    del B_x
    anyspec = pl.BlockSpec(memory_space=pl.ANY)
    out = pl.pallas_call(
        _kernel,
        out_shape=jax.ShapeDtypeStruct((S, D), bf16),
        in_specs=[anyspec] * 7,
        out_specs=anyspec,
        scratch_shapes=[
            pltpu.VMEM((S, D), bf16),
            pltpu.VMEM((D, D), bf16),
            pltpu.VMEM((D + 2 * DH, D), bf16),
            pltpu.VMEM((D, D), bf16),
            pltpu.VMEM((F, D), bf16),
            pltpu.VMEM((F, D), bf16),
            pltpu.VMEM((S, D), bf16),
            pltpu.VMEM((S, D), bf16),
            pltpu.VMEM((NU, DH, TQ), bf16),
            pltpu.VMEM((NU, DH, TQ), f32),
            pltpu.VMEM((NU, TQ), f32),
            pltpu.VMEM((NI, G, TQ), f32),
            pltpu.VMEM((NB * 8, DE), u32),
            pltpu.VMEM((S, DE), bf16),
            pltpu.VMEM((NV, DE), bf16),
            pltpu.VMEM((DH, NV + NX, 128), f32),
            pltpu.VMEM((DH, S), f32),
            pltpu.VMEM((NU, DH, TQ), bf16),
            pltpu.VMEM((2, NV, TQ), f32),
            pltpu.VMEM((ROT * 16, TQ), f32),
            pltpu.VMEM((NU, NX, TQ), f32),
            pltpu.VMEM((S, D), f32),
            pltpu.VMEM((TQ, D), f32),
            pltpu.VMEM((TQ, F), bf16),
            pltpu.VMEM((DH, TQ), f32),
            pltpu.VMEM((8, 128), u32),
            pltpu.SemaphoreType.DMA((NT,)),
            pltpu.SemaphoreType.DMA((6,)),
            pltpu.SemaphoreType.DMA((len(OSEG),)),
        ],
        compiler_params=pltpu.CompilerParams(vmem_limit_bytes=100 * 1024 * 1024),
    )(A_x.reshape(S, D), A_wq, A_wk.T, A_wv.T, A_wo, B_w1.T, B_w2)
    return out.reshape(1, S, D)
```

```python
import math

import jax
import jax.numpy as jnp
import numpy as np
from jax import lax
import jax.experimental.pallas as pl
import jax.experimental.pallas.tpu as pltpu

S, D, H, DH, F = 2048, 512, 32, 16, 1376
TQ = 512
NT = S // TQ
NU = NT * H
KC = 128
NK = S // KC
NC = TQ // 128
DE = 32
QSCALE = (DH ** -0.5) * math.log2(math.e)
UP = 1.0 + 2.0 ** -6
L_MIN = 2.0 ** -60
EPS = 1e-5
f32, bf16, u32 = jnp.float32, jnp.bfloat16, jnp.uint32
NT_DIMS = (((1,), (1,)), ((), ()))
TN_DIMS = (((0,), (0,)), ((), ()))
FT = [(a, min(a + 128, F)) for a in range(0, F, 128)]

G = 8
NVL = [16, 16, 32, 16, 16, 16, 16, 32] + [16] * 8
NXL = [16, 0, 0, 0, 0] * 3 + [0]
LEAD = 8
ROT = 8
S1 = 8
HALF = 24
W1FRAC, F0, F1, FHALF = 0.5, 0.01, 0.03, 12
LN_AHEAD = 3
XA, XB = 3, 8
OSPLIT = 4


def _offsets(counts, div):
    return [int(v) // div for v in np.concatenate([[0], np.cumsum(counts)])]


GOFF, XOFF = _offsets(NVL, 8), _offsets(NXL, 8)
NV, NX = int(sum(NVL)), int(sum(NXL))
NBL = [(KC - v - w) // 16 for v, w in zip(NVL, NXL)]
BOFF = _offsets(NBL, 1)
NB = BOFF[-1]
NG, NGX = NV // 8, NX // 8
TILE_OF_GROUP = [j for j in range(NK) for _ in range(NVL[j] // 8)]
ALLP = [(g, r0 + r, c) for g in range(G) for r0 in range(0, NG, 2) for c in range(NC) for r in range(2)]
_LO, _HI = ROT * 8, (G * NB + ROT - S1) * 8
PTS = [min(_HI - 1, int(_LO + n * (_HI - _LO) / len(ALLP))) for n in range(len(ALLP))]
NI = NU // G
XP = [(h, r0 + r, c) for h in range(H) for r0 in range(0, NGX, 2) for c in range(NC) for r in range(2)]
XN1 = int(len(XP) * W1FRAC) // 2 * 2
XP1 = [int((F0 + (1 - F0) * n / XN1) * len(FT) * (TQ // 8)) for n in range(XN1)]
XP2 = [int((1 - F1) * n / (len(XP) - XN1) * len(FT) * (TQ // 8) * NC) for n in range(len(XP) - XN1)]
OSEG = ([(t * TQ, (t + 1) * TQ) for t in range(NT - 1)]
        + [((NT - 1) * TQ + k * (TQ // OSPLIT), (NT - 1) * TQ + (k + 1) * (TQ // OSPLIT)) for k in range(OSPLIT)])


def _kernel(x_hbm, wq_hbm, wkt_hbm, wvt_hbm, wo_hbm, w1t_hbm, w2_hbm, o_hbm,
            x_ref, wq_ref, wt_ref, wo_ref, w1t_ref, w2_ref, o_ref,
            xn_ref, qt_ref, qf_ref, nrm_ref, bias_ref, kx_ref, kn_ref, kv_ref, kb_ref,
            vt_ref, ot_ref, pvs_ref, pre_ref, px_ref, y_ref, ya_ref, h_ref, zf_ref, z_ref,
            sem_x, sem_w, sem_o):
    x_cp = [pltpu.make_async_copy(x_hbm.at[pl.ds(a, b - a)], x_ref.at[pl.ds(a, b - a)], sem_x.at[n])
            for n, (a, b) in enumerate([(0, XA * 128), (XA * 128, XB * 128), (XB * 128, S)])]
    w_cp = [pltpu.make_async_copy(a, b, sem_w.at[i]) for i, (a, b) in enumerate(
        [(wq_hbm, wq_ref), (wkt_hbm, wt_ref.at[pl.ds(D, DH)]), (wvt_hbm, wt_ref.at[pl.ds(D + DH, DH)]),
         (w1t_hbm, w1t_ref), (w2_hbm, w2_ref), (wo_hbm, wo_ref)])]
    for c in w_cp[:3]:
        c.start()
    x_cp[0].start()
    zf_ref[...] = jnp.zeros(zf_ref.shape, f32)
    z_ref[...] = jnp.zeros(z_ref.shape, u32)

    row16 = lax.broadcasted_iota(jnp.int32, (DH, TQ), 0)
    row8 = lax.broadcasted_iota(jnp.int32, (8, TQ), 0)

    def layernorm(s, lk=None):
        x = x_ref[s * 128:(s + 1) * 128, :].astype(f32)
        if lk is not None:
            never = jnp.concatenate([z_ref[...] != 0] * 16, axis=0)
            x = jnp.concatenate([jnp.where(never, lk, x[:, 0:128]), x[:, 128:]], axis=1)
        mu = jnp.mean(x, axis=-1, keepdims=True)
        xc = x - mu
        var = jnp.mean(xc * xc, axis=-1, keepdims=True)
        xn_ref[s * 128:(s + 1) * 128, :] = (xc * lax.rsqrt(var + EPS)).astype(bf16)

    def proj_kv(t):
        xn = xn_ref[t * TQ:(t + 1) * TQ, :]
        r = lax.dot_general(wt_ref[D:D + 2 * DH, :], xn, NT_DIMS, preferred_element_type=f32)
        kt = r[0:DH].astype(bf16).astype(f32)
        vt_ref[:, t * TQ:(t + 1) * TQ] = r[DH:].astype(bf16).astype(f32)
        k2 = jnp.sum(kt * kt, axis=0, keepdims=True)
        ones_row = jnp.where(row16 == 0, 1.0, 0.0).astype(f32)
        ke = jnp.concatenate([kt, ones_row], axis=0).T
        kn_ref[t * TQ:(t + 1) * TQ, :] = ke.astype(bf16)
        for jj in range(TQ // KC):
            j = t * (TQ // KC) + jj
            for b in range(NBL[j]):
                src = jj * KC + NVL[j] + NXL[j] + 16 * (NBL[j] - 1 - b)
                kk = jnp.concatenate([ke[src + 8:src + 16, :], ke[src:src + 8, :]], axis=0)
                kx_ref[8 * (BOFF[j] + b): 8 * (BOFF[j] + b) + 8, :] = pltpu.bitcast(kk.astype(bf16), u32)
            if NVL[j]:
                kv_ref[GOFF[j] * 8: GOFF[j] * 8 + NVL[j], :] = ke[jj * KC: jj * KC + NVL[j], :].astype(bf16)
            for r0 in range(0, NVL[j] + NXL[j], 8):
                kv = ke[jj * KC + r0: jj * KC + r0 + 8, :]
                dst = GOFF[j] * 8 + r0 if r0 < NVL[j] else NV + XOFF[j] * 8 + r0 - NVL[j]
                for d in range(DH):
                    kb_ref[d, dst:dst + 8, :] = jnp.broadcast_to(kv[:, d:d + 1], (8, 128))
        return k2

    def proj_q(s):
        t, a = s // NC, (s % NC) * 128
        xn = xn_ref[s * 128:(s + 1) * 128, :]
        r = lax.dot_general(wt_ref[0:D, :], xn, NT_DIMS, preferred_element_type=f32)
        qb = (r * QSCALE).astype(bf16)
        qf = qb.astype(f32).reshape(H, DH, 128)
        qt_ref[t * H:(t + 1) * H, :, a:a + 128] = qb.reshape(H, DH, 128)
        qf_ref[t * H:(t + 1) * H, :, a:a + 128] = qf
        nrm_ref[t * H:(t + 1) * H, a:a + 128] = jnp.sum(qf * qf, axis=1)
        return r

    def q_ext(it, g):
        brow = jnp.broadcast_to(bias_ref[it, g:g + 1, :], (8, TQ))
        blk = jnp.concatenate([jnp.where(row8 == 0, brow, 0.0), jnp.zeros((8, TQ), f32)], axis=0)
        return jnp.concatenate([qt_ref[G * it + g], blk.astype(bf16)], axis=0)

    for c in w_cp[:3]:
        c.wait()
    x_cp[0].wait()
    x_cp[1].start()
    wt_ref[0:D, :] = wq_ref[...].T
    k2 = None
    outs = {}
    nln = nkv = 0
    for s in range(NT * NC):
        if s == XA - 1:
            x_cp[1].wait()
            x_cp[2].start()
            outs = {}
        if s == XB - 1:
            x_cp[2].wait()
            for c in w_cp[3:]:
                c.start()
            outs = {}
        avail = XA if s < XA - 1 else (XB if s < XB - 1 else NT * NC)
        while nln < avail and nln - LN_AHEAD < max(s, 1):
            lk = outs.get(nln - LN_AHEAD)
            if lk is not None:
                lk = jnp.concatenate([lk[32 * n:32 * n + 8] for n in range(16)], axis=0)
            layernorm(nln, lk)
            nln += 1
        while nkv < NT and (nkv + 1) * NC - 1 <= s and s not in (XA - 2, XB - 2):
            kk2 = proj_kv(nkv)
            k2 = kk2 if k2 is None else jnp.maximum(k2, kk2)
            nkv += 1
        assert nln > s
        outs[s] = proj_q(s)
    assert nkv == NT
    kscale = jnp.sqrt(jnp.max(k2, axis=1, keepdims=True)) * (-UP)
    for t in range(NT):
        bias = (jnp.sqrt(nrm_ref[t * H:(t + 1) * H, :]) * kscale).astype(bf16).astype(f32)
        for k in range(H // G):
            bias_ref[t * (H // G) + k] = bias[k * G:(k + 1) * G]

    def vpu_probs(never, it, g, krow, c, lk, lk2=None):
        u = G * it + g
        acc = jnp.broadcast_to(bias_ref[it, g:g + 1, c * 128:(c + 1) * 128], (16, 128))
        acc = jnp.where(never, jnp.concatenate(lk, axis=0), acc)
        for d in range(DH):
            if d == DH // 2 and lk2 is not None:
                acc = jnp.where(never, jnp.concatenate(lk2, axis=0), acc)
            qb = jnp.broadcast_to(qf_ref[u, d:d + 1, c * 128:(c + 1) * 128], (16, 128))
            acc = acc + kb_ref[d, krow * 8:krow * 8 + 16, :] * qb
        return jnp.exp2(acc)

    def kblocks(b0, b1):
        return pltpu.bitcast(kx_ref[8 * b0:8 * b1, :], bf16)

    pvs_ref[0] = jnp.exp2(jnp.dot(kv_ref[...], q_ext(0, 0), preferred_element_type=f32))
    pre_ref[...] = jnp.exp2(jnp.dot(kblocks(0, ROT), q_ext(0, 0), preferred_element_type=f32))

    w_cp[3].wait()
    w_cp[4].wait()

    def ffn(t, carry):
        rows = pl.ds(pl.multiple_of(t * TQ, TQ), TQ)
        never = jnp.concatenate([z_ref[...] != 0] * 2, axis=0)
        xn = xn_ref[rows, :]
        k = [0]

        hs, parts = {}, {}
        nv1, nv2 = TQ // 8, TQ // 8 * NC

        def emit(lk, lk2=None):
            h, r, c = XP[k[0]]
            assert XP[k[0] + 1] == (h, r + 1, c)
            px_ref[t * H + h, r * 8:r * 8 + 16, c * 128:(c + 1) * 128] = vpu_probs(
                never, t * (H // G) + h // G, h % G, NG + r, c, lk, lk2)
            k[0] += 2

        def h_vreg(p):
            hv = hs[p // nv1][(p % nv1) * 8:(p % nv1) * 8 + 8, :]
            if hv.shape[1] < 128:
                hv = jnp.concatenate([hv, hv[:, 0:128 - hv.shape[1]]], axis=1)
            return hv

        def part_vreg(p):
            rg, cc = (p % nv2) // NC, p % NC
            return parts[p // nv2][rg * 8:rg * 8 + 8, cc * 128:(cc + 1) * 128]

        for n, (a, b) in enumerate(FT):
            h = lax.dot_general(xn, w1t_ref[a:b, :], NT_DIMS, preferred_element_type=f32)
            hh = h * 0.5
            h_ref[:, a:b] = (hh + hh * jnp.tanh(hh)).astype(bf16)
            hs[n] = h
            while k[0] < XN1 and XP1[k[0] + 1] // nv1 <= n:
                emit([h_vreg(p) for p in XP1[k[0]:k[0] + 2]])
        for n, (a, b) in enumerate(FT):
            part = jnp.dot(h_ref[:, a:b], w2_ref[a:b, :], preferred_element_type=f32)
            if n == 0:
                ya_ref[...] = x_ref[rows, :].astype(f32) + part
            elif n == len(FT) - 1:
                y_ref[rows, :] = ya_ref[...] + part
            else:
                ya_ref[...] += part
            parts[n] = part
            while k[0] < len(XP) and (XP2[k[0] + 1 - XN1] + FHALF) // nv2 <= n:
                ps = XP2[k[0] - XN1:k[0] - XN1 + 2]
                emit([part_vreg(p) for p in ps], [part_vreg(p + FHALF) for p in ps])
        assert k[0] == len(XP)
        return carry

    lax.fori_loop(0, NT, ffn, 0)

    def stage(i, bad):
        L = [None] * G
        ACC = [None] * G
        Q = [None] * (G + 1)
        PM, SS = {}, {}
        done_v = set()
        st = dict(nextp=0, pos=ROT, bad=bad)
        never = jnp.concatenate([z_ref[...] != 0] * 2, axis=0)
        inext = jnp.minimum(i + 1, NI - 1)

        def score_vreg(x):
            hf, cc = (x % 8) // 4, x % 4
            return SS[x // 8][8 * hf:8 * hf + 8, cc * 128:(cc + 1) * 128]

        def emit_pieces():
            while st["nextp"] < len(ALLP):
                g, r, c = ALLP[st["nextp"]]
                xs = PTS[st["nextp"]:st["nextp"] + 2]
                if ((xs[1] + HALF) // 8) not in SS or (g >= 1 and (g - 1, TILE_OF_GROUP[r + 1]) not in done_v):
                    break
                it2, g2 = (i, g + 1) if g + 1 < G else (inext, 0)
                pvs_ref[g2 % 2, r * 8:r * 8 + 16, c * 128:(c + 1) * 128] = vpu_probs(
                    never, it2, g2, r, c, [score_vreg(x) for x in xs], [score_vreg(x + HALF) for x in xs])
                st["nextp"] += 2

        def score(g, b0, b1):
            if Q[g] is None:
                Q[g] = q_ext(i, g) if g < G else q_ext(inext, 0)
            s = jnp.dot(kblocks(b0, b1), Q[g], preferred_element_type=f32)
            p = jnp.exp2(s)
            if g == G:
                pre_ref[16 * b0:16 * b1, :] = p
            for b in range(b0, b1):
                PM[(g, b)] = p[16 * (b - b0):16 * (b - b0) + 16]
                SS[g * NB + b] = s[16 * (b - b0):16 * (b - b0) + 16]

        def pv(g, j):
            blocks = [(pre_ref[16 * b:16 * b + 16, :] if (g == 0 and b < ROT) else PM.pop((g, b)))
                      for b in range(BOFF[j], BOFF[j + 1])]
            blocks = [y for x in blocks for y in (x[0:8], x[8:16])]
            if g >= 1:
                assert all((g - 1, r, c) in ALLP[:st["nextp"]]
                           for r in range(GOFF[j], GOFF[j + 1]) for c in range(NC))
            rows = [pvs_ref[g % 2, r * 8:r * 8 + 8, :] for r in range(GOFF[j], GOFF[j + 1])]
            rows += [px_ref[G * i + g, r * 8:r * 8 + 8, :] for r in range(XOFF[j], XOFF[j + 1])]
            for x in blocks + rows[::-1]:
                L[g] = x if L[g] is None else L[g] + x
            pb = jnp.concatenate(rows + blocks[::-1], axis=0)
            o = jnp.dot(vt_ref[:, j * KC:(j + 1) * KC], pb, preferred_element_type=f32,
                        precision=lax.Precision.DEFAULT)
            if ACC[g] is None:
                ACC[g] = zf_ref[...]
            ACC[g] = ACC[g] + o
            if j == NK - 1:
                lsum = jnp.sum(L[g], axis=0, keepdims=True)
                ot_ref[G * i + g] = (ACC[g] / lsum).astype(bf16)
                st["bad"] = jnp.where(lsum >= L_MIN, st["bad"], 1.0)
            done_v.add((g, j))
            emit_pieces()

        def issue_to(p1):
            p1 = min(p1, G * NB + ROT)
            while st["pos"] < p1:
                g = st["pos"] // NB
                e = min(p1, (g + 1) * NB)
                score(g, st["pos"] - g * NB, e - g * NB)
                st["pos"] = e
                emit_pieces()

        for g in range(G):
            for j in range(NK):
                issue_to(g * NB + BOFF[j + 1] + LEAD)
                pv(g, j)
        issue_to(G * NB + ROT)
        assert st["nextp"] == len(ALLP)
        return st["bad"]

    bad = lax.fori_loop(0, NI, stage, jnp.zeros((1, TQ), f32))

    @pl.when(jnp.max(bad) > 0.0)
    def _():
        def unit(u, c):
            s = jnp.dot(kn_ref[:, 0:DH], qt_ref[u], preferred_element_type=f32)
            m = jnp.max(s, axis=0, keepdims=True)
            p = jnp.exp2(s - m)
            l = jnp.sum(p, axis=0, keepdims=True)
            o = jnp.dot(vt_ref[...].astype(bf16), p.astype(bf16), preferred_element_type=f32)
            ot_ref[u] = (o / l).astype(bf16)
            return c
        lax.fori_loop(0, NU, unit, 0)

    w_cp[5].wait()
    o_cp = [pltpu.make_async_copy(o_ref.at[pl.ds(a, b - a)], o_hbm.at[pl.ds(a, b - a)], sem_o.at[n])
            for n, (a, b) in enumerate(OSEG)]
    for n, (a, b) in enumerate(OSEG):
        t = a // TQ
        ot = ot_ref[t * H:(t + 1) * H, :, a - t * TQ:b - t * TQ].reshape(H * DH, b - a)
        att = lax.dot_general(ot, wo_ref[...], TN_DIMS, preferred_element_type=f32)
        o_ref[a:b, :] = (y_ref[a:b, :] + att).astype(bf16)
        o_cp[n].start()
    for c in o_cp:
        c.wait()


@jax.jit
def pallas_parallel_sum__grouped_kv_mqa__dense_activation_silu__prompt_kernel(
    A_x: jax.Array,
    A_wq: jax.Array,
    A_wk: jax.Array,
    A_wv: jax.Array,
    A_wo: jax.Array,
    B_x: jax.Array,
    B_w1: jax.Array,
    B_w2: jax.Array,
):
    del B_x
    anyspec = pl.BlockSpec(memory_space=pl.ANY)
    out = pl.pallas_call(
        _kernel,
        out_shape=jax.ShapeDtypeStruct((S, D), bf16),
        in_specs=[anyspec] * 7,
        out_specs=anyspec,
        scratch_shapes=[
            pltpu.VMEM((S, D), bf16),
            pltpu.VMEM((D, D), bf16),
            pltpu.VMEM((D + 2 * DH, D), bf16),
            pltpu.VMEM((D, D), bf16),
            pltpu.VMEM((F, D), bf16),
            pltpu.VMEM((F, D), bf16),
            pltpu.VMEM((S, D), bf16),
            pltpu.VMEM((S, D), bf16),
            pltpu.VMEM((NU, DH, TQ), bf16),
            pltpu.VMEM((NU, DH, TQ), f32),
            pltpu.VMEM((NU, TQ), f32),
            pltpu.VMEM((NI, G, TQ), f32),
            pltpu.VMEM((NB * 8, DE), u32),
            pltpu.VMEM((S, DE), bf16),
            pltpu.VMEM((NV, DE), bf16),
            pltpu.VMEM((DH, NV + NX, 128), f32),
            pltpu.VMEM((DH, S), f32),
            pltpu.VMEM((NU, DH, TQ), bf16),
            pltpu.VMEM((2, NV, TQ), f32),
            pltpu.VMEM((ROT * 16, TQ), f32),
            pltpu.VMEM((NU, NX, TQ), f32),
            pltpu.VMEM((S, D), f32),
            pltpu.VMEM((TQ, D), f32),
            pltpu.VMEM((TQ, F), bf16),
            pltpu.VMEM((DH, TQ), f32),
            pltpu.VMEM((8, 128), u32),
            pltpu.SemaphoreType.DMA((3,)),
            pltpu.SemaphoreType.DMA((6,)),
            pltpu.SemaphoreType.DMA((len(OSEG),)),
        ],
        compiler_params=pltpu.CompilerParams(vmem_limit_bytes=100 * 1024 * 1024),
    )(A_x.reshape(S, D), A_wq, A_wk.T, A_wv.T, A_wo, B_w1.T, B_w2)
    return out.reshape(1, S, D)
```
